```python
import jax
import jax.numpy as jnp

def _softmax(x, axis=-1):
    return jax.nn.softmax(x, axis=axis)

def _gelu(x):
    return jax.nn.gelu(x, approximate=True)

def _silu(x):
    return jax.nn.silu(x)

def _sigmoid(x):
    return jax.nn.sigmoid(x)

def _layernorm(x, axis=-1, eps=1e-05):
    m = jnp.mean(x, axis=axis, keepdims=True)
    v = jnp.var(x, axis=axis, keepdims=True)
    return (x - m) / jnp.sqrt(v + eps)

def _scatter_add(tgt, idx, src, axis=0):
    return tgt.at[idx].add(src)

def _segment_sum(src, seg, n):
    return jax.ops.segment_sum(src, seg, n)

class _Rng:

    def __init__(self, key):
        self._k = key

    def _next(self):
        self._k, sub = jax.random.split(self._k)
        return sub

    def normal(self, shape):
        return jax.random.normal(self._next(), shape, dtype=jnp.bfloat16)

    def randint(self, lo, hi, shape):
        return jax.random.randint(self._next(), shape, lo, hi, dtype=jnp.int32)

    def uniform(self, shape, lo=0.0, hi=1.0):
        return jax.random.uniform(self._next(), shape, jnp.bfloat16, lo, hi)

    def permutation(self, n):
        return jax.random.permutation(self._next(), n)
kernel_name = 'concat_heads__memory_aug_recurrent_mem_tr__spectral_gfnet__prompt'

def setup_inputs():
    _rng = _Rng(jax.random.key(int.from_bytes(__import__("os").urandom(4), "little")))
    _w = lambda a: (lambda t: t.astype(jnp.bfloat16) if jnp.issubdtype(t.dtype, jnp.floating) else t)(jnp.asarray(a))

    def _A_setup():
        B, S, Dm = (1, 2048, 1024)
        H, Dh = (32, 128)
        M, seg = (8, 32)
        seg = min(seg, S)
        S = S // seg * seg
        return {'x': _w((lambda *s: _rng.normal(s) * 0.05)(B, S, Dm)), 'mem0': _w((lambda *s: _rng.normal(s) * 0.05)(B, M, Dm)), 'Wq': _w((lambda *s: _rng.normal(s) * 0.05)(Dm, H, Dh) * Dm ** (-0.5)), 'Wk': _w((lambda *s: _rng.normal(s) * 0.05)(Dm, H, Dh) * Dm ** (-0.5)), 'Wv': _w((lambda *s: _rng.normal(s) * 0.05)(Dm, H, Dh) * Dm ** (-0.5)), 'Wo': _w((lambda *s: _rng.normal(s) * 0.05)(H, Dh, Dm) * (H * Dh) ** (-0.5)), 'seg_len': seg}
    _A_in = _A_setup()

    def _B_setup():
        B, S, D = (1, 2048, 1024)
        Df = D // 2 + 1
        return {'x': _w((lambda *s: _rng.normal(s) * 0.05)(B, S, D)), 'w_r': _w((lambda *s: _rng.normal(s) * 0.05)(S, Df) * 0.02), 'w_i': _w((lambda *s: _rng.normal(s) * 0.05)(S, Df) * 0.02)}
    _B_in = _B_setup()
    return {'A_x': _A_in['x'], 'A_mem0': _A_in['mem0'], 'A_Wq': _A_in['Wq'], 'A_Wk': _A_in['Wk'], 'A_Wv': _A_in['Wv'], 'A_Wo': _A_in['Wo'], 'A_seg_len': _A_in['seg_len'], 'B_x': _B_in['x'], 'B_w_r': _B_in['w_r'], 'B_w_i': _B_in['w_i']}

def reference(A_x, A_mem0, A_Wq, A_Wk, A_Wv, A_Wo, A_seg_len, B_x, B_w_r, B_w_i):

    def _A_ref(x, mem0, Wq, Wk, Wv, Wo, seg_len):
        B, S, Dm = x.shape
        H, Dh = (Wq.shape[1], Wq.shape[2])
        M = mem0.shape[1]
        scale = Dh ** (-0.5)
        n_seg = S // seg_len
        L = M + seg_len
        idx = jnp.arange(L)
        mask = (idx[:, None] < M) | (idx[:, None] >= idx[None, :])
        mem = mem0
        outs = []
        for s in range(n_seg):
            xs = x[:, s * seg_len:(s + 1) * seg_len, :].copy()
            h = jnp.concatenate([mem, xs], axis=1)
            q = jnp.einsum('btd,dhe->bhte', h, Wq)
            k = jnp.einsum('btd,dhe->bhte', h, Wk)
            v = jnp.einsum('btd,dhe->bhte', h, Wv)
            scores = jnp.einsum('bhqe,bhke->bhqk', q, k) * scale
            scores = jnp.where(mask[None, None], scores, -1000000000.0)
            p = _softmax(scores, axis=-1)
            o = jnp.einsum('bhqk,bhke->bhqe', p, v)
            o = jnp.einsum('bhte,hed->btd', o, Wo)
            mem = o[:, :M, :].copy()
            outs.append(o[:, M:, :])
        return jnp.concatenate(outs, axis=1)

    def _B_ref(x, w_r, w_i):
        B, S, D = x.shape
        X = (lambda x, axes=(-2, -1): jnp.fft.rfft2(x.astype(jnp.float32), axes=axes))(x, axes=(-2, -1))
        W = w_r + 1j * w_i
        X = X * W
        y = (lambda x, s, axes=(-2, -1): jnp.fft.irfft2(x, s=s, axes=axes).astype(jnp.bfloat16))(X, (S, D), axes=(-2, -1))
        return y
    a = _A_ref(A_x, A_mem0, A_Wq, A_Wk, A_Wv, A_Wo, A_seg_len)
    b = _B_ref(B_x, B_w_r, B_w_i)
    return jnp.concatenate([a, b], axis=-1)
```

```python
import math
import numpy as np
import jax
import jax.numpy as jnp
from jax import lax
from jax.experimental import pallas as pl
from jax.experimental.pallas import tpu as pltpu

S, DM, H, DH, M, SEG = 2048, 1024, 32, 128, 8, 32
L = M + SEG
NSEG = S // SEG
N1, N2 = 64, 32
f32, bf16, u32 = jnp.float32, jnp.bfloat16, jnp.uint32
SK1, SK2 = 1, 2


def _consts():
    d = np.arange(DM)[:, None].astype(np.float64)
    k = np.arange(DM // 2)[None, :].astype(np.float64)
    ang = 2 * np.pi * ((d * k) % DM) / DM
    fd = np.concatenate([np.cos(ang), -np.sin(ang)], axis=1)
    fd[:, DM // 2] = np.cos(np.pi * d[:, 0])
    wt = np.full((DM,), 2.0)
    wt[0] = 1.0
    wt[DM // 2] = 1.0
    fdi = fd.T * wt[:, None] / (S * DM)
    n2 = np.arange(N2)[:, None, None]
    k1 = np.arange(N1)[None, :, None]
    n1 = np.arange(N1)[None, None, :]
    a = 2 * np.pi * ((k1 * (N2 * n1 + n2)) % S) / S
    c, s = np.cos(a), -np.sin(a)
    g = np.concatenate([np.concatenate([c, -s], axis=2), np.concatenate([s, c], axis=2)], axis=1)
    gi = np.transpose(g, (0, 2, 1))
    cast = lambda t: np.ascontiguousarray(t).astype(np.float32).astype(jnp.bfloat16)
    return cast(fd), cast(fdi), cast(g), cast(gi)


def _tw(z, k, n):
    k %= n
    zr, zi = z
    if k == 0:
        return z
    if 4 * k == n:
        return (zi, -zr)
    if 2 * k == n:
        return (-zr, -zi)
    if 4 * k == 3 * n:
        return (-zi, zr)
    c, s = math.cos(2 * math.pi * k / n), -math.sin(2 * math.pi * k / n)
    if (8 * k) % n == 0:
        r = math.sqrt(0.5)
        if 8 * k == n:
            return ((zr + zi) * r, (zi - zr) * r)
        if 8 * k == 3 * n:
            return ((zi - zr) * r, (zr + zi) * (-r))
    return (zr * c - zi * s, zr * s + zi * c)


def _fft(x):
    n = len(x)
    if n == 1:
        return x
    if n == 2:
        (ar, ai), (br, bi) = x
        return [(ar + br, ai + bi), (ar - br, ai - bi)]
    e, o1, o3 = _fft(x[0::2]), _fft(x[1::4]), _fft(x[3::4])
    out = [None] * n
    q = n // 4
    for k in range(q):
        t1, t3 = _tw(o1[k], k, n), _tw(o3[k], 3 * k, n)
        sr, si = t1[0] + t3[0], t1[1] + t3[1]
        dr, di = t1[0] - t3[0], t1[1] - t3[1]
        out[k] = (e[k][0] + sr, e[k][1] + si)
        out[k + 2 * q] = (e[k][0] - sr, e[k][1] - si)
        out[k + q] = (e[k + q][0] + di, e[k + q][1] - dr)
        out[k + 3 * q] = (e[k + q][0] - di, e[k + q][1] + dr)
    return out


def _ifft(x):
    return [(b, a) for a, b in _fft([(b, a) for a, b in x])]


def _kernel(x_hbm, mem_ref, wq_hbm, wk_hbm, wv_hbm, wo_hbm, bx_hbm, wr_hbm, wi_hbm,
            fd_hbm, fdi_hbm, g_hbm, gi_hbm, out_hbm,
            xbuf, wbuf, wobuf, hbuf, obuf, ybuf,
            bxbuf, wrbuf, wibuf, fdbuf, fdibuf, gbuf, gibuf, zbuf, sems):
    def start(src, dst, i):
        c = pltpu.make_async_copy(src, dst, sems.at[i])
        c.start()
        return c

    bxu = bx_hbm.bitcast(u32)
    c_fd = start(fd_hbm, fdbuf, 0)
    c_g = start(g_hbm, gbuf, 0)
    c_bx = [start(bxu.at[:, m, :], bxbuf.at[m], 1) for m in range(N2 // 2)]
    c_w = [start(wr_hbm, wrbuf, 2), start(wi_hbm, wibuf, 2)]
    c_inv = [start(fdi_hbm, fdibuf, 3), start(gi_hbm, gibuf, 3)]
    c_a = [start(x_hbm, xbuf, 4)]
    for t, w in enumerate((wq_hbm, wk_hbm, wv_hbm)):
        wu = w.bitcast(u32)
        for j in range(H // 2):
            c_a.append(start(wu.at[:, :, j, :], wbuf.at[t, j], 4))
    wou = wo_hbm.bitcast(u32)
    for n in range(DM // 128):
        c_a.append(start(wou.at[:, pl.ds(n * 128, 128)], wobuf.at[n], 4))

    c_fd.wait()
    c_g.wait()
    for c in c_bx:
        c.wait()
    lane0 = lax.broadcasted_iota(jnp.int32, (N1, 128), 1) == 0

    def fwd(m, _):
        w = bxbuf[m]
        lo = pltpu.bitcast(w << 16, f32)
        hi = pltpu.bitcast(w & jnp.uint32(0xFFFF0000), f32)
        z = jnp.dot(jnp.concatenate([lo, hi], axis=0), fdbuf[...], preferred_element_type=f32)
        for p in range(2):
            zr = z[p * N1:(p + 1) * N1, :512]
            zi = z[p * N1:(p + 1) * N1, 512:]
            zi0 = zi[:, :128]
            top = jnp.concatenate([zr, jnp.where(lane0, zi0, 0.0)], axis=1)
            bot = jnp.concatenate([jnp.where(lane0, 0.0, zi0), zi[:, 128:], jnp.zeros((N1, 128), f32)], axis=1)
            rhs = jnp.concatenate([top, bot], axis=0).astype(bf16)
            zbuf[2 * m + p] = jnp.dot(gbuf[2 * m + p], rhs, preferred_element_type=f32)
        return 0
    lax.fori_loop(0, N2 // 2, fwd, 0)

    for c in c_w:
        c.wait()

    def mid_tile(g, t, last):
        r = pl.multiple_of(g * 8, 8)
        ln = pl.ds(t * 128, 128) if last else pl.ds(pl.multiple_of(t * 128, 128), 128)
        y = [(zbuf[n, pl.ds(r, 8), ln], zbuf[n, pl.ds(N1 + r, 8), ln]) for n in range(N2)]
        y = _fft(y)
        for k in range(N2):
            rows = pl.ds(pl.multiple_of(k * N1 + r, 8), 8)
            if last:
                wr = jnp.broadcast_to(wrbuf[rows, 512:513].astype(f32), (8, 128))
                wi = jnp.broadcast_to(wibuf[rows, 512:513].astype(f32), (8, 128))
            else:
                wr = wrbuf[rows, ln].astype(f32)
                wi = wibuf[rows, ln].astype(f32)
            yr, yi = y[k]
            y[k] = (yr * wr - yi * wi, yr * wi + yi * wr)
        y = _ifft(y)
        for n in range(N2):
            zbuf[n, pl.ds(r, 8), ln] = y[n][0]
            zbuf[n, pl.ds(N1 + r, 8), ln] = y[n][1]

    def mid(i, _):
        mid_tile(i // 4, i % 4, False)
        return 0
    lax.fori_loop(0, 32, mid, 0)

    def mid_last(g, _):
        mid_tile(g, 4, True)
        return 0
    lax.fori_loop(0, 8, mid_last, 0)

    for c in c_inv:
        c.wait()

    def inv(m, _):
        rows = []
        for p in range(2):
            z = jnp.dot(gibuf[2 * m + p], zbuf[2 * m + p].astype(bf16), preferred_element_type=f32)
            zi0 = jnp.where(lane0, z[:N1, 512:], z[N1:, :128])
            rows.append(jnp.concatenate([z[:N1, :512], zi0, z[N1:, 128:512]], axis=1))
        y = jnp.dot(jnp.concatenate(rows, axis=0), fdibuf[...], preferred_element_type=f32)
        y = pltpu.bitcast(y.astype(bf16).astype(f32), u32)
        bxbuf[m] = (y[:N1] >> 16) | y[N1:]
        return 0
    lax.fori_loop(0, N2 // 2, inv, 0)
    outu = out_hbm.bitcast(u32)
    c_ob = [start(bxbuf.at[m], outu.at[:, m, pl.ds(DM, DM)], 1) for m in range(N2 // 2)]

    for c in c_a:
        c.wait()

    def relayout(i, _):
        t, j = i // 16, i % 16
        for g in range(64):
            a = wbuf[t, j, g, pl.ds(0, 8, stride=2), :]
            b = wbuf[t, j, g, pl.ds(1, 8, stride=2), :]
            wbuf[t, j, g, 0:8, :] = (a & jnp.uint32(0xFFFF)) | (b << 16)
            wbuf[t, j, g, 8:16, :] = (a >> 16) | (b & jnp.uint32(0xFFFF0000))
        return 0
    lax.fori_loop(0, 48, relayout, 0)

    hbuf[0:M, :] = mem_ref[...].astype(f32)
    row = lax.broadcasted_iota(jnp.int32, (L, 128), 0)
    col = lax.broadcasted_iota(jnp.int32, (L, 128), 1)
    mask = (col < L) & ((row < M) | (row >= col))
    scale = DH ** -0.5

    def getw(t, h):
        w = wbuf[t, h // 2, :, pl.ds((h % 2) * 8, 8), :]
        return pltpu.bitcast(w.reshape(DM // 2, DH), bf16)

    def step(s, _):
        hbuf[M:L, :] = xbuf[s].astype(f32)
        st = {}
        for i in range(H + SK2):
            if i < H:
                hv = hbuf[...]
                k = jnp.dot(hv, getw(1, i), preferred_element_type=f32)
                q = jnp.dot(hv, getw(0, i), preferred_element_type=f32)
                v = jnp.dot(hv, getw(2, i), preferred_element_type=f32)
                zpad = jnp.zeros((128 - L, DH), f32)
                kp = jnp.concatenate([k, zpad], axis=0).astype(bf16)
                vp = jnp.concatenate([v, zpad], axis=0).astype(bf16)
                st[i] = [q, kp, vp]
            h = i - SK1
            if 0 <= h < H:
                q, kp, vp = st[h]
                sc = lax.dot_general(q, kp, (((1,), (1,)), ((), ())), preferred_element_type=f32) * scale
                sc = jnp.where(mask, sc, -1e30)
                e = jnp.exp(sc - jnp.max(sc, axis=1, keepdims=True))
                st[h] = [e, jnp.sum(e, axis=1, keepdims=True), vp]
            h = i - SK2
            if 0 <= h < H:
                e, l, vp = st.pop(h)
                obuf[:, h * DH:(h + 1) * DH] = jnp.dot(e, vp, preferred_element_type=f32) / l
        ov = obuf[...]
        for n in range(DM // 128):
            y = jnp.dot(ov, pltpu.bitcast(wobuf[n], bf16), preferred_element_type=f32)
            hbuf[0:M, n * 128:(n + 1) * 128] = y[0:M].astype(bf16).astype(f32)
            ybuf[s, :, n * 128:(n + 1) * 128] = y[M:L].astype(bf16)
        return 0
    lax.fori_loop(0, NSEG, step, 0)
    c_oa = start(ybuf, out_hbm.at[:, :, pl.ds(0, DM)], 0)
    for c in c_ob:
        c.wait()
    c_oa.wait()


@jax.jit
def pallas_concat_heads__memory_aug_recurrent_mem_tr__spectral_gfnet__prompt_kernel(
        A_x, A_mem0, A_Wq, A_Wk, A_Wv, A_Wo, A_seg_len, B_x, B_w_r, B_w_i):
    del A_seg_len
    fd, fdi, g, gi = _consts()
    rw = lambda w: w.reshape(DM // 16, 16, H, DH)
    anyspec = pl.BlockSpec(memory_space=pl.ANY)
    vm = pltpu.VMEM
    out = pl.pallas_call(
        _kernel,
        out_shape=jax.ShapeDtypeStruct((N1, N2, 2 * DM), bf16),
        in_specs=[anyspec, pl.BlockSpec(memory_space=vm)] + [anyspec] * 11,
        out_specs=anyspec,
        scratch_shapes=[
            vm((NSEG, SEG, DM), bf16), vm((3, H // 2, DM // 16, 16, DH), u32), vm((DM // 128, H * DH // 2, 128), u32),
            vm((L, DM), f32), vm((L, H * DH), f32), vm((NSEG, SEG, DM), bf16),
            vm((N2 // 2, N1, DM), u32), vm((S, DM // 2 + 1), bf16), vm((S, DM // 2 + 1), bf16),
            vm((DM, DM), bf16), vm((DM, DM), bf16), vm((N2, 128, 128), bf16), vm((N2, 128, 128), bf16),
            vm((N2, 128, 640), f32), pltpu.SemaphoreType.DMA((5,))],
        compiler_params=pltpu.CompilerParams(vmem_limit_bytes=110 * 1024 * 1024),
    )(A_x.reshape(NSEG, SEG, DM), A_mem0.reshape(M, DM), rw(A_Wq), rw(A_Wk), rw(A_Wv),
      A_Wo.reshape(H * DH, DM), B_x.reshape(N1, N2, DM), B_w_r, B_w_i, fd, fdi, g, gi)
    return out.reshape(1, S, 2 * DM)
```

```python
import math
import numpy as np
import jax
import jax.numpy as jnp
from jax import lax
from jax.experimental import pallas as pl
from jax.experimental.pallas import tpu as pltpu

S, DM, H, DH, M, SEG = 2048, 1024, 32, 128, 8, 32
L = M + SEG
NSEG = S // SEG
N1, N2 = 64, 32
F1, F2, X1, NP = 4, 12, 4, 8
f32, bf16, u32 = jnp.float32, jnp.bfloat16, jnp.uint32
import os
CFG = int(os.environ.get("CFG", 0))
G, SK1, SK2, TAIL = [
    (4, 1, 2, {32: [(0, 8, 0, 8)], 33: [(8, 24, 0, 8)], -1: [(24, 28, 0, 8), (28, 32, 0, 8)]}),
    (1, 1, 2, {32: [(0, 8, 0, 4)], 33: [(0, 8, 4, 8)], -1: [(8, 24, 0, 8), (24, 32, 0, 8)]}),
    (2, 1, 2, {32: [(0, 8, 0, 4)], 33: [(0, 8, 4, 8), (8, 16, 0, 4)], -1: [(8, 16, 4, 8), (16, 32, 0, 8)]}),
    (4, 1, 3, {32: [(0, 8, 0, 8)], 33: [(8, 16, 0, 8)], 34: [(16, 24, 0, 8)], -1: [(24, 28, 0, 8), (28, 32, 0, 8)]}),
][CFG]


_CLS = ((0, 4), (1, 7), (2, 6), (3, 5))
_BETA = {0: 1, 4: -1, 1: -1j, 7: 1j, 2: -1j, 6: 1j, 3: 1j, 5: -1j}


def _consts():
    b = np.arange(128)[:, None]
    fd = np.zeros((4, 256, 256))
    fdi = np.zeros((4, 256, 256))
    for t, cls in enumerate(_CLS):
        k = np.concatenate([c + 8 * np.arange(64) for c in cls])[None, :]
        beta = np.concatenate([np.full(64, _BETA[c], np.complex128) for c in cls])[None, :]
        e = np.exp(-2j * np.pi * ((b * k) % DM) / DM)
        m = np.concatenate([e, beta * e], axis=0)
        re, im = m.real.copy(), m.imag.copy()
        wt = np.full((256,), 2.0)
        if t == 0:
            im[:, 0] = np.tile(np.cos(np.pi * b[:, 0]), 2)
            wt[0] = wt[128] = 1.0
        fd[t] = np.concatenate([re, im], axis=1)
        fdi[t] = fd[t].T * wt[:, None] / (S * DM)
    n2 = np.arange(N2)[:, None, None]
    k1 = np.arange(N1)[None, :, None]
    n1 = np.arange(N1)[None, None, :]
    a = 2 * np.pi * ((k1 * (N2 * n1 + n2)) % S) / S
    c, s = np.cos(a), -np.sin(a)
    g = np.concatenate([np.concatenate([c, -s], axis=2), np.concatenate([s, c], axis=2)], axis=1)
    gi = np.transpose(g, (0, 2, 1))
    cast = lambda t: np.ascontiguousarray(t).astype(np.float32).astype(jnp.bfloat16)
    return cast(fd), cast(fdi), cast(g), cast(gi)


def _tw(z, k, n):
    k %= n
    zr, zi = z
    if k == 0:
        return z
    if 4 * k == n:
        return (zi, -zr)
    if 2 * k == n:
        return (-zr, -zi)
    if 4 * k == 3 * n:
        return (-zi, zr)
    c, s = math.cos(2 * math.pi * k / n), -math.sin(2 * math.pi * k / n)
    if (8 * k) % n == 0:
        r = math.sqrt(0.5)
        if 8 * k == n:
            return ((zr + zi) * r, (zi - zr) * r)
        if 8 * k == 3 * n:
            return ((zi - zr) * r, (zr + zi) * (-r))
    return (zr * c - zi * s, zr * s + zi * c)


def _fft(x):
    n = len(x)
    if n == 1:
        return x
    if n == 2:
        (ar, ai), (br, bi) = x
        return [(ar + br, ai + bi), (ar - br, ai - bi)]
    e, o1, o3 = _fft(x[0::2]), _fft(x[1::4]), _fft(x[3::4])
    out = [None] * n
    q = n // 4
    for k in range(q):
        t1, t3 = _tw(o1[k], k, n), _tw(o3[k], 3 * k, n)
        sr, si = t1[0] + t3[0], t1[1] + t3[1]
        dr, di = t1[0] - t3[0], t1[1] - t3[1]
        out[k] = (e[k][0] + sr, e[k][1] + si)
        out[k + 2 * q] = (e[k][0] - sr, e[k][1] - si)
        out[k + q] = (e[k + q][0] + di, e[k + q][1] - dr)
        out[k + 3 * q] = (e[k + q][0] - di, e[k + q][1] + dr)
    return out


def _ifft(x):
    return [(b, a) for a, b in _fft([(b, a) for a, b in x])]


def _loop(name, lo, hi, fn):
    with jax.named_scope(name):
        lax.fori_loop(lo, hi, lambda i, _: fn(i, _), 0)


def _wait(name, cs):
    with jax.named_scope(name):
        for c in cs:
            c.wait()


def _lo(w):
    return pltpu.bitcast(w << 16, f32)


def _hi(w):
    return pltpu.bitcast(w & jnp.uint32(0xFFFF0000), f32)


def _kernel(x_hbm, mem_hbm, wq_hbm, wk_hbm, wv_hbm, wo_hbm, bx_hbm, wr_hbm, wi_hbm,
            fd_hbm, fdi_hbm, g_hbm, gi_hbm, out_hbm,
            xbuf, membuf, wbuf, wobuf, hbuf, obuf, ybuf,
            bxbuf, wtbuf, wnbuf, wpbuf, fdbuf, fdibuf, gbuf, gibuf, zbuf, xqbuf, qbuf, sems):
    def start(src, dst, i):
        c = pltpu.make_async_copy(src, dst, sems.at[i])
        c.start()
        return c

    bxu = bx_hbm.bitcast(u32)
    c_f = [start(fd_hbm, fdbuf, 0), start(g_hbm, gbuf, 0)]
    c_f += [start(bxu.at[:, m, :], bxbuf.at[m], 0) for m in range(F1)]
    c_f2 = [start(bxu.at[:, m, :], bxbuf.at[m], 1) for m in range(F1, N2 // 2)]
    c_w = []
    for i, w in enumerate((wr_hbm, wi_hbm)):
        wu = w.at[pl.ds(0, DM // 2), :].bitcast(u32)
        c_w += [start(wu.at[:, pl.ds(j * 128, 128)], wtbuf.at[i, j], 2) for j in range(S // 128)]
        c_w.append(start(w.at[pl.ds(DM // 2, 1), :], wnbuf.at[i], 2))
    c_inv = [start(fdi_hbm, fdibuf, 3), start(gi_hbm, gibuf, 3)]

    def load_w(t):
        wu = (wq_hbm, wk_hbm, wv_hbm)[t].bitcast(u32)
        return [start(wu.at[:, :, j, :], wbuf.at[t, j], 4 + t) for j in range(H // 2)]

    lane0 = lax.broadcasted_iota(jnp.int32, (N1, 128), 1) == 0
    rt = math.sqrt(0.5)

    def fwd(m, with_w):
        w = bxbuf[m]
        xs = [jnp.concatenate([_lo(w[:, a * 128:(a + 1) * 128]), _hi(w[:, a * 128:(a + 1) * 128])], axis=0)
              for a in range(8)]
        u0, u1, u2, u3 = xs[0] + xs[4], xs[0] - xs[4], xs[2] + xs[6], xs[2] - xs[6]
        u4, u5, u6, u7 = xs[1] + xs[5], xs[1] - xs[5], xs[3] + xs[7], xs[3] - xs[7]
        d, e = (u5 - u7) * rt, (u5 + u7) * rt
        ab = ((u0 + u2, u4 + u6), (u1 + d, u3 + e), (u0 - u2, u4 - u6), (u1 - d, u3 - e))
        z = [jnp.dot(jnp.concatenate(ab[t], axis=1).astype(bf16), fdbuf[t], preferred_element_type=f32)
             for t in range(4)]
        if with_w:
            for j in range(4):
                jt = 4 * (m - F2) + j
                ln = pl.ds(pl.multiple_of(jt * 128, 128), 128)
                for i in range(2):
                    p = [wtbuf[i, jt, pl.ds(c, 64, stride=4), :] for c in range(4)]
                    lo, hi = jnp.uint32(0xFFFF), jnp.uint32(0xFFFF0000)
                    wpbuf[2 * i, ln, :] = jnp.concatenate([p[0], (p[2] & lo) | (p[3] & hi)], axis=0).T
                    wpbuf[2 * i + 1, ln, :] = jnp.concatenate([p[1], (p[3] & lo) | (p[2] & hi)], axis=0).T
                nr = pltpu.bitcast(wnbuf[0, :, ln].astype(f32), u32)
                ni = pltpu.bitcast(wnbuf[1, :, ln].astype(f32), u32)
                wpbuf[4, ln, :] = jnp.broadcast_to((nr >> 16) | ni, (128, 128)).T
        for p in range(2):
            rows = slice(p * N1, (p + 1) * N1)
            zi0 = z[0][rows, 128:]
            top = [z[t][rows, :128] for t in range(4)] + [jnp.where(lane0, zi0, 0.0)]
            bot = [jnp.where(lane0, 0.0, zi0)] + [z[t][rows, 128:] for t in range(1, 4)] + [jnp.zeros((N1, 128), f32)]
            rhs = jnp.concatenate([jnp.concatenate(top, axis=1), jnp.concatenate(bot, axis=1)], axis=0)
            y = jnp.dot(gbuf[2 * m + p], rhs.astype(bf16), preferred_element_type=f32)
            for t in range(5):
                zbuf[2 * m + p, t] = y[:, t * 128:(t + 1) * 128]
        return 0

    _wait('wc_f', c_f)
    _loop('fwd1', 0, F1, lambda m, _: fwd(m, False))
    c_q = load_w(0) + [start(x_hbm.at[:, pl.ds(SEG - NP, NP), :], xqbuf, 4)]
    _wait('wc_f2', c_f2)
    _loop('fwd2', F1, F2, lambda m, _: fwd(m, False))
    c_k = load_w(1)
    _wait('wc_w', c_w)
    _loop('fwd3', F2, N2 // 2, lambda m, _: fwd(m, True))

    c_v = load_w(2)
    wou = wo_hbm.bitcast(u32)
    c_o = [start(wou.at[:, pl.ds(n * 128, 128)], wobuf.at[n], 7) for n in range(DM // 128)]
    c_o.append(start(mem_hbm, membuf, 7))
    c_o.append(start(x_hbm.at[pl.ds(0, X1)], xbuf.at[pl.ds(0, X1)], 7))

    def mid_tile(g, t, getw):
        r = pl.multiple_of(g * 8, 8)
        y = _fft([(zbuf[n, t, pl.ds(r, 8), :], zbuf[n, t, pl.ds(N1 + r, 8), :]) for n in range(N2)])
        for k in range(N2):
            wr, wi = getw(pl.ds(pl.multiple_of(k * N1 + r, 8), 8))
            yr, yi = y[k]
            y[k] = (yr * wr - yi * wi, yr * wi + yi * wr)
        y = _ifft(y)
        for n in range(N2):
            zbuf[n, t, pl.ds(r, 8), :] = y[n][0]
            zbuf[n, t, pl.ds(N1 + r, 8), :] = y[n][1]

    def mid(i, _):
        g, pr = i // 2, i % 2
        mid_tile(g, 2 * pr, lambda rows: (_lo(wpbuf[pr, rows, :]), _lo(wpbuf[2 + pr, rows, :])))
        mid_tile(g, 2 * pr + 1, lambda rows: (_hi(wpbuf[pr, rows, :]), _hi(wpbuf[2 + pr, rows, :])))
        return 0
    _loop('mid', 0, 16, mid)

    def mid_last(g, _):
        mid_tile(g, 4, lambda rows: (_lo(wpbuf[4, rows, :]), _hi(wpbuf[4, rows, :])))
        return 0
    _loop('mid_last', 0, 8, mid_last)

    _wait('wc_inv', c_inv)

    def inv(m, _):
        zs = []
        for p in range(2):
            rhs = jnp.concatenate([zbuf[2 * m + p, t] for t in range(5)], axis=1).astype(bf16)
            zs.append(jnp.dot(gibuf[2 * m + p], rhs, preferred_element_type=f32))
        ab = []
        for t in range(4):
            ln = slice(t * 128, (t + 1) * 128)
            re = [z[:N1, ln] for z in zs]
            im = [jnp.where(lane0, z[:N1, 512:], z[N1:, ln]) if t == 0 else z[N1:, ln] for z in zs]
            lhs = jnp.concatenate([jnp.concatenate(re, axis=0), jnp.concatenate(im, axis=0)], axis=1)
            v = jnp.dot(lhs.astype(bf16), fdibuf[t], preferred_element_type=f32)
            ab.append((v[:, :128], v[:, 128:]))
        (p_, q_), (a1, b1), (a2, b2), (a3, b3) = ab
        u0, u2, u4, u6 = p_ + a2, p_ - a2, q_ + b2, q_ - b2
        u1, u3, d, e = a1 + a3, b1 + b3, (a1 - a3) * rt, (b1 - b3) * rt
        u5, u7 = e + d, e - d
        ys = (u0 + u1, u4 + u5, u2 + u3, u6 + u7, u0 - u1, u4 - u5, u2 - u3, u6 - u7)
        for a in range(8):
            y = pltpu.bitcast(ys[a].astype(bf16).astype(f32), u32)
            bxbuf[m, :, a * 128:(a + 1) * 128] = (y[:N1] >> 16) | y[N1:]
        return 0
    _loop('inv', 0, N2 // 2, inv)
    outu = out_hbm.bitcast(u32)

    def getw(t, h):
        w = wbuf[t, h // 2, :, pl.ds((h % 2) * 8, 8), :]
        return pltpu.bitcast(w.reshape(DM // 2, DH), bf16)

    def relayout(t, j):
        for g in range(64):
            a = wbuf[t, j, g, pl.ds(0, 8, stride=2), :]
            b = wbuf[t, j, g, pl.ds(1, 8, stride=2), :]
            wbuf[t, j, g, 0:8, :] = (a & jnp.uint32(0xFFFF)) | (b << 16)
            wbuf[t, j, g, 8:16, :] = (a >> 16) | (b & jnp.uint32(0xFFFF0000))

    def pre(j, t, nxt):
        xq = xqbuf[...].astype(f32).reshape(NSEG * NP, DM)
        for p in range(2):
            w = wbuf[0, j, :, pl.ds(p * 8, 8), :]
            w = pltpu.bitcast(w.reshape(DM // 2, DH), bf16)
            qbuf[2 * j + p] = jnp.dot(xq, w, preferred_element_type=f32)
        if nxt:
            relayout(0, j + 1)
        relayout(t, 2 * (j % 8))
        relayout(t, 2 * (j % 8) + 1)
        return 0

    _wait('wc_q', c_q)
    relayout(0, 0)
    _wait('wc_k', c_k)
    _loop('pre1', 0, 8, lambda j, _: pre(j, 1, True))
    _wait('wc_v', c_v)
    _loop('pre2', 8, 15, lambda j, _: pre(j, 2, True))
    pre(15, 2, False)
    c_x = start(x_hbm.at[pl.ds(X1, NSEG - X1)], xbuf.at[pl.ds(X1, NSEG - X1)], 8)
    c_out = [start(bxbuf.at[m], outu.at[:, m, pl.ds(DM, DM)], 0) for m in range(N2 // 2)]
    _wait('wc_o', c_o)

    hbuf[0:M, :] = membuf[...].astype(f32)
    row = lax.broadcasted_iota(jnp.int32, (L, 128), 0)
    col = lax.broadcasted_iota(jnp.int32, (L, 128), 1)
    mask = (col < L) & ((row < M) | (row >= col))
    scale = DH ** -0.5

    def ycopy(s):
        return pltpu.make_async_copy(ybuf.at[s], out_hbm.at[s, :, pl.ds(0, DM)], sems.at[1])

    def step(s, _):
        hbuf[M:L, :] = xbuf[s].astype(f32)
        st = {}
        acc = [None] * (DM // 128)

        def proj(h):
            hv = hbuf[...]
            k = jnp.dot(hv, getw(1, h), preferred_element_type=f32)
            q = jnp.dot(hv[:L - NP], getw(0, h), preferred_element_type=f32)
            q = jnp.concatenate([q, qbuf[h, pl.ds(pl.multiple_of(s * NP, NP), NP), :]], axis=0)
            v = jnp.dot(hv, getw(2, h), preferred_element_type=f32)
            zpad = jnp.zeros((128 - L, DH), f32)
            st[h] = (q, jnp.concatenate([k, zpad], axis=0).astype(bf16),
                     jnp.concatenate([v, zpad], axis=0).astype(bf16))

        def scores(h):
            q, kp, vp = st[h]
            sc = lax.dot_general(q, kp, (((1,), (1,)), ((), ())), preferred_element_type=f32) * scale
            sc = jnp.where(mask, sc, -1e30)
            e = jnp.exp(sc - jnp.max(sc, axis=1, keepdims=True))
            st[h] = (e, jnp.sum(e, axis=1, keepdims=True), vp)

        def pv(h):
            e, l, vp = st.pop(h)
            obuf[:, h * DH:(h + 1) * DH] = jnp.dot(e, vp, preferred_element_type=f32) / l

        def outproj(h0, h1, n0, n1):
            for n in range(n0, n1):
                w = pltpu.bitcast(wobuf[n, h0 * DH // 2:h1 * DH // 2, :], bf16)
                y = jnp.dot(obuf[:, h0 * DH:h1 * DH], w, preferred_element_type=f32)
                acc[n] = y if acc[n] is None else acc[n] + y
                if h1 == H:
                    hbuf[0:M, n * 128:(n + 1) * 128] = acc[n][0:M].astype(bf16).astype(f32)
                    ybuf[s, :, n * 128:(n + 1) * 128] = acc[n][M:L].astype(bf16)

        for i in range(H + SK2):
            if i < H:
                proj(i)
            for part in TAIL.get(i, ()):
                outproj(*part)
            for fn, e_ in ((scores, i - SK1), (pv, i - SK2)):
                if 0 <= e_ < H and (e_ + 1) % G == 0:
                    for h in range(e_ - G + 1, e_ + 1):
                        fn(h)
        for part in TAIL[-1]:
            outproj(*part)
        ycopy(s).start()
        return 0

    def phase(ph, _):
        @pl.when(ph == 1)
        def _():
            c_x.wait()
        lax.fori_loop(ph * X1, X1 + ph * (NSEG - X1), step, 0)
        return 0
    _loop('step', 0, 2, phase)
    _wait('wc_out', c_out)
    pltpu.make_async_copy(ybuf, ybuf, sems.at[1]).wait()


@jax.jit
def pallas_concat_heads__memory_aug_recurrent_mem_tr__spectral_gfnet__prompt_kernel(
        A_x, A_mem0, A_Wq, A_Wk, A_Wv, A_Wo, A_seg_len, B_x, B_w_r, B_w_i):
    del A_seg_len
    fd, fdi, g, gi = _consts()
    rw = lambda w: w.reshape(DM // 16, 16, H, DH)
    hbm = pl.BlockSpec(memory_space=pltpu.HBM)
    vm = pltpu.VMEM
    args = (A_x.reshape(NSEG, SEG, DM), A_mem0.reshape(M, DM), rw(A_Wq), rw(A_Wk), rw(A_Wv),
            A_Wo.reshape(H * DH, DM), B_x.reshape(N1, N2, DM), B_w_r.T, B_w_i.T, fd, fdi, g, gi)
    out = pl.pallas_call(
        _kernel,
        out_shape=jax.ShapeDtypeStruct((N1, N2, 2 * DM), bf16),
        in_specs=[hbm] * 13,
        out_specs=hbm,
        scratch_shapes=[
            vm((NSEG, SEG, DM), bf16), vm((M, DM), bf16),
            vm((3, H // 2, DM // 16, 16, DH), u32), vm((DM // 128, H * DH // 2, 128), u32),
            vm((L, DM), f32), vm((L, H * DH), f32), vm((NSEG, SEG, DM), bf16),
            vm((N2 // 2, N1, DM), u32), vm((2, S // 128, DM // 4, 128), u32), vm((2, 1, S), bf16), vm((5, S, 128), u32),
            vm((4, 256, 256), bf16), vm((4, 256, 256), bf16), vm((N2, 128, 128), bf16), vm((N2, 128, 128), bf16),
            vm((N2, 5, 128, 128), f32), vm((NSEG, NP, DM), bf16), vm((H, NSEG * NP, DH), f32),
            pltpu.SemaphoreType.DMA((9,))],
        compiler_params=pltpu.CompilerParams(vmem_limit_bytes=110 * 1024 * 1024),
    )(*[pltpu.with_memory_space_constraint(jnp.asarray(t), pltpu.HBM) for t in args])
    return out.reshape(1, S, 2 * DM)
```

```python
import functools
import math
import numpy as np
import jax
import jax.numpy as jnp
from jax import lax
from jax.experimental import pallas as pl
from jax.experimental.pallas import tpu as pltpu

S, DM, H, DH, M, SEG = 2048, 1024, 32, 128, 8, 32
L = M + SEG
NSEG = S // SEG
N1, N2 = 64, 32
F1, F2, X1, NP = 4, 12, 4, 8
NPAIR, NK = H // 2, 16
f32, bf16, u32 = jnp.float32, jnp.bfloat16, jnp.uint32
import os
CFG = int(os.environ.get("CFG", 0))


PSTEP = int(os.environ.get('PSTEP', 64))


DIST = int(os.environ.get('DIST', 2))


UF, UM, UI, US = [int(c) for c in os.environ.get('U', '1112')]


def _schedule():
    ev = []
    for h in range(H):
        ev.append(("proj", h))
        g, r = h // 4 - 1, h % 4
        if g >= 0:
            if r == 0:
                ev += [("qk", 4 * g + i) for i in range(4)]
            elif r == 3:
                ev += [("pv", 4 * g + i) for i in range(4)]
            else:
                ev += [("soft", 4 * g + 2 * r - 2), ("soft", 4 * g + 2 * r - 1)]
    o = lambda h0, h1, ns: [("out", h0, h1, n) for n in ns]
    if CFG == 0:
        ev += o(0, 8, (0, 1)) + [("qk", h) for h in range(28, 32)] + o(0, 8, (2, 3))
        for i in range(4):
            ev += [("soft", 28 + i)] + o(0, 8, (4 + i,))
        ev += o(8, 16, range(4)) + [("pv", h) for h in range(28, 32)] + o(8, 16, range(4, 8)) + o(16, 32, range(8))
    elif CFG == 1:
        ev += o(0, 16, (0,)) + [("qk", h) for h in range(28, 32)] + o(0, 16, (1,))
        for i in range(4):
            ev += [("soft", 28 + i)] + o(0, 16, (2 + i,))
        ev += o(0, 16, (6,)) + [("pv", h) for h in range(28, 32)] + o(0, 16, (7,)) + o(16, 32, range(8))
    elif CFG == 2:
        ev += o(0, 28, (0,)) + [("qk", h) for h in range(28, 32)] + o(0, 28, (1,))
        ev += [("soft", 28), ("soft", 29)] + o(0, 28, (2,)) + [("soft", 30), ("soft", 31)] + o(0, 28, (3,))
        ev += [("pv", h) for h in range(28, 32)] + o(0, 28, (4,)) + o(28, 32, range(5)) + o(0, 32, range(5, 8))
    return ev


_CLS = ((0, 4), (1, 7), (2, 6), (3, 5))
_BETA = {0: 1, 4: -1, 1: -1j, 7: 1j, 2: -1j, 6: 1j, 3: 1j, 5: -1j}


def _consts():
    b = np.arange(128)[:, None]
    fd = np.zeros((4, 256, 256))
    fdi = np.zeros((4, 256, 256))
    for t, cls in enumerate(_CLS):
        k = np.concatenate([c + 8 * np.arange(64) for c in cls])[None, :]
        beta = np.concatenate([np.full(64, _BETA[c], np.complex128) for c in cls])[None, :]
        e = np.exp(-2j * np.pi * ((b * k) % DM) / DM)
        m = np.concatenate([e, beta * e], axis=0)
        re, im = m.real.copy(), m.imag.copy()
        wt = np.full((256,), 2.0)
        if t == 0:
            im[:, 0] = np.tile(np.cos(np.pi * b[:, 0]), 2)
            wt[0] = wt[128] = 1.0
        fd[t] = np.concatenate([re, im], axis=1)
        fdi[t] = fd[t].T * wt[:, None] / (S * DM)
    n2 = np.arange(N2)[:, None, None]
    k1 = np.arange(N1)[None, :, None]
    n1 = np.arange(N1)[None, None, :]
    a = 2 * np.pi * ((k1 * (N2 * n1 + n2)) % S) / S
    c, s = np.cos(a), -np.sin(a)
    g = np.concatenate([np.concatenate([c, -s], axis=2), np.concatenate([s, c], axis=2)], axis=1)
    gi = np.transpose(g, (0, 2, 1))
    cast = lambda t: np.ascontiguousarray(t).astype(np.float32).astype(jnp.bfloat16)
    return cast(fd), cast(fdi), cast(g), cast(gi)


def _tw(z, k, n):
    k %= n
    zr, zi = z
    if k == 0:
        return z
    if 4 * k == n:
        return (zi, -zr)
    if 2 * k == n:
        return (-zr, -zi)
    if 4 * k == 3 * n:
        return (-zi, zr)
    c, s = math.cos(2 * math.pi * k / n), -math.sin(2 * math.pi * k / n)
    if (8 * k) % n == 0:
        r = math.sqrt(0.5)
        if 8 * k == n:
            return ((zr + zi) * r, (zi - zr) * r)
        if 8 * k == 3 * n:
            return ((zi - zr) * r, (zr + zi) * (-r))
    return (zr * c - zi * s, zr * s + zi * c)


def _fft(x):
    n = len(x)
    if n == 1:
        return x
    if n == 2:
        (ar, ai), (br, bi) = x
        return [(ar + br, ai + bi), (ar - br, ai - bi)]
    e, o1, o3 = _fft(x[0::2]), _fft(x[1::4]), _fft(x[3::4])
    out = [None] * n
    q = n // 4
    for k in range(q):
        t1, t3 = _tw(o1[k], k, n), _tw(o3[k], 3 * k, n)
        sr, si = t1[0] + t3[0], t1[1] + t3[1]
        dr, di = t1[0] - t3[0], t1[1] - t3[1]
        out[k] = (e[k][0] + sr, e[k][1] + si)
        out[k + 2 * q] = (e[k][0] - sr, e[k][1] - si)
        out[k + q] = (e[k + q][0] + di, e[k + q][1] - dr)
        out[k + 3 * q] = (e[k + q][0] - di, e[k + q][1] + dr)
    return out


def _ifft(x):
    return [(b, a) for a, b in _fft([(b, a) for a, b in x])]


def _loop(name, lo, hi, fn, unroll=1, pre=None):
    def body(i, _):
        if pre is not None:
            pre(i)
        for j in range(unroll):
            fn(lo + i * unroll + j, 0)
        return 0
    with jax.named_scope(name):
        lax.fori_loop(0, (hi - lo) // unroll, body, 0)


def _wait(name, cs):
    with jax.named_scope(name):
        for c in cs:
            c.wait()


def _lo(w):
    return pltpu.bitcast(w << 16, f32)


def _hi(w):
    return pltpu.bitcast(w & jnp.uint32(0xFFFF0000), f32)


def _kernel(x_hbm, mem_hbm, wq_hbm, wk_hbm, wv_hbm, wo_hbm, bx_hbm, wr_hbm, wi_hbm,
            fd_hbm, fdi_hbm, g_hbm, gi_hbm, out_hbm,
            xbuf, membuf, wbuf, wobuf, hbuf, obuf, ybuf,
            bxbuf, wtbuf, wnbuf, wpbuf, fdbuf, fdibuf, gbuf, gibuf, zbuf, xqbuf, xfbuf, qkbuf, sems):
    def start(src, dst, i):
        c = pltpu.make_async_copy(src, dst, sems.at[i])
        c.start()
        return c

    bxu = bx_hbm.bitcast(u32)

    def load_f(m0, m1, sem):
        gs = pl.ds(2 * m0, 2 * (m1 - m0))
        return ([start(g_hbm.at[gs], gbuf.at[gs], sem)]
                + [start(bxu.at[:, m, :], bxbuf.at[m], sem) for m in range(m0, m1)])

    c_f = [start(fd_hbm, fdbuf, 0)] + load_f(0, 2, 0)
    c_f2 = [load_f(2, 4, 1), load_f(4, 8, 13), load_f(8, 16, 14)]
    def load_w(t, j0, j1, sem):
        wu = (wq_hbm, wk_hbm, wv_hbm)[t].bitcast(u32)
        return [start(wu.at[:, :, j, :], wbuf.at[t * NPAIR + j], sem) for j in range(j0, j1)]

    def getw(u, p):
        w = wbuf[u, :, pl.ds(p * 8, 8), :]
        return pltpu.bitcast(w.reshape(DM // 2, DH), bf16)

    def relayout(u, half=None):
        for g in (range(64) if half is None else [32 * half + i for i in range(32)]):
            a = wbuf[u, g, pl.ds(0, 8, stride=2), :]
            b = wbuf[u, g, pl.ds(1, 8, stride=2), :]
            wbuf[u, g, 0:8, :] = (a & jnp.uint32(0xFFFF)) | (b << 16)
            wbuf[u, g, 8:16, :] = (a >> 16) | (b & jnp.uint32(0xFFFF0000))

    def wait_if(cond, cs):
        @pl.when(cond)
        def _():
            for c in cs:
                c.wait()

    lane0 = lax.broadcasted_iota(jnp.int32, (N1, 128), 1) == 0
    rt = math.sqrt(0.5)

    def fwd(m, _):
        w = bxbuf[m]
        xs = [jnp.concatenate([_lo(w[:, a * 128:(a + 1) * 128]), _hi(w[:, a * 128:(a + 1) * 128])], axis=0)
              for a in range(8)]
        u0, u1, u2, u3 = xs[0] + xs[4], xs[0] - xs[4], xs[2] + xs[6], xs[2] - xs[6]
        u4, u5, u6, u7 = xs[1] + xs[5], xs[1] - xs[5], xs[3] + xs[7], xs[3] - xs[7]
        d, e = (u5 - u7) * rt, (u5 + u7) * rt
        ab = ((u0 + u2, u4 + u6), (u1 + d, u3 + e), (u0 - u2, u4 - u6), (u1 - d, u3 - e))
        z = [jnp.dot(jnp.concatenate(ab[t], axis=1).astype(bf16), fdbuf[t], preferred_element_type=f32)
             for t in range(4)]
        for p in range(2):
            rows = slice(p * N1, (p + 1) * N1)
            zi0 = z[0][rows, 128:]
            top = [z[t][rows, :128] for t in range(4)] + [jnp.where(lane0, zi0, 0.0)]
            bot = [jnp.where(lane0, 0.0, zi0)] + [z[t][rows, 128:] for t in range(1, 4)] + [jnp.zeros((N1, 128), f32)]
            rhs = jnp.concatenate([jnp.concatenate(top, axis=1), jnp.concatenate(bot, axis=1)], axis=0)
            y = jnp.dot(gbuf[2 * m + p], rhs.astype(bf16), preferred_element_type=f32)
            for t in range(5):
                for c in range(2):
                    zbuf[t, :, 2 * m + p, c] = y[c * N1:(c + 1) * N1, t * 128:(t + 1) * 128].reshape(8, 8, 128)
        return 0

    def permute_w(jt):
        def put(i, v):
            v = v.T
            for c in range(2):
                wpbuf[i, :, 2 * jt + c] = v[c * N1:(c + 1) * N1].reshape(8, 8, 128)
        ln = pl.ds(pl.multiple_of(jt * 128, 128), 128)
        for i in range(2):
            p = [wtbuf[i, jt, pl.ds(c, 64, stride=4), :] for c in range(4)]
            lo, hi = jnp.uint32(0xFFFF), jnp.uint32(0xFFFF0000)
            put(2 * i, jnp.concatenate([p[0], (p[2] & lo) | (p[3] & hi)], axis=0))
            put(2 * i + 1, jnp.concatenate([p[1], (p[3] & lo) | (p[2] & hi)], axis=0))
        nr = pltpu.bitcast(wnbuf[0, :, ln].astype(f32), u32)
        ni = pltpu.bitcast(wnbuf[1, :, ln].astype(f32), u32)
        put(4, jnp.broadcast_to((nr >> 16) | ni, (128, 128)))

    c_q = [[start(x_hbm.at[:, pl.ds(SEG - NP, NP), :], xqbuf, 4)] + load_w(0, 0, 3, 4)]
    c_w = []
    for i, w in enumerate((wr_hbm, wi_hbm)):
        wu = w.at[pl.ds(0, DM // 2), :].bitcast(u32)
        c_w += [start(wu.at[:, pl.ds(j * 128, 128)], wtbuf.at[i, j], 2) for j in range(S // 128)]
        c_w.append(start(w.at[pl.ds(DM // 2, 1), :], wnbuf.at[i], 2))

    def fwd_waits(i):
        for c, m in zip(c_f2, (2, 4, 8)):
            wait_if(i == m, c)
    _wait('wc_f', c_f)
    _loop('fwd', 0, N2 // 2, fwd, 1, fwd_waits)
    c_q += [load_w(0, 3, 5, 5), load_w(0, 5, 10, 6), load_w(0, 10, 16, 15)]
    c_inv = [start(fdi_hbm, fdibuf, 3), start(gi_hbm, gibuf, 3)]
    c_k = [load_w(1, 0, 9, 9), load_w(1, 9, 16, 10)]
    def mid_pieces(g, t, res):
        def lds(ns):
            z = [(zbuf[t, g, n, 0], zbuf[t, g, n, 1]) for n in ns]
            if len(res) >= DIST:
                z[0] = (jnp.where(t < 0, res[-DIST], z[0][0]), z[0][1])
                z[1] = (z[1][0], jnp.where(t < 0, res[-DIST], z[1][1]))
            return z
        nyq = t // 4
        ir, ii = t // 2 + 2 * nyq, t // 2 + 2
        sr = (16 * (1 - t % 2)).astype(u32)
        si = (16 * (1 - t % 2 - nyq)).astype(u32)
        half = lambda w, sh: pltpu.bitcast((w << sh) & jnp.uint32(0xFFFF0000), f32)

        def st(n, z):
            zbuf[t, g, n, 0] = z[0]
            zbuf[t, g, n, 1] = z[1]

        def p1(b):
            y = _fft(lds([4 * a + b for a in range(8)]))
            for ka in range(8):
                st(4 * ka + b, _tw(y[ka], b * ka, N2))

        def p2(ka):
            y = _fft(lds([4 * ka + b for b in range(4)]))
            for kb in range(4):
                wr, wi = half(wpbuf[ir, g, ka + 8 * kb], sr), half(wpbuf[ii, g, ka + 8 * kb], si)
                yr, yi = y[kb]
                y[kb] = (yr * wr - yi * wi, yr * wi + yi * wr)
            y = _ifft(y)
            for b in range(4):
                st(4 * ka + b, _tw(y[b], -b * ka, N2))

        def p3(b):
            y = _ifft(lds([4 * ka + b for ka in range(8)]))
            for a in range(8):
                st(4 * a + b, y[a])

        P = functools.partial
        return [P(p1, b) for b in range(4)] + [P(p2, k) for k in range(8)] + [P(p3, b) for b in range(4)]

    def pre_pieces(u, step, res):
        def piece(p, r):
            y = jnp.dot(xfbuf[u % 2, r:r + step, :], getw(u // 2, p), preferred_element_type=f32)
            res.append(y[0:8])
            qkbuf[u // 2, p, u % 2, r:r + step, :] = y
        return [functools.partial(piece, p, r) for p in range(2) for r in range(0, NSEG * NP // 2, step)]

    def mid(u, _):
        res = []
        mp = mid_pieces((u - 8) // 5, (u - 8) % 5, res)
        pp = pre_pieces(u, PSTEP, res)
        k = len(mp) // len(pp)
        for c, p in enumerate(pp):
            p()
            for f in mp[c * k:(c + 1) * k]:
                f()
        relayout(u // 2 + 1, u % 2)
        return 0

    def pre(u, with_w):
        for p in pre_pieces(u, 256, []):
            p()
        if with_w:
            for j in range(4):
                permute_w(4 * (u - 4) + j)
        relayout(u // 2 + 1, u % 2)

    _wait('wc_q', c_q[0])
    xfbuf[...] = xqbuf[...].astype(f32).reshape(2, NSEG * NP // 2, DM)
    relayout(0)
    _loop('preA', 0, 4, lambda u, _: pre(u, False))
    c_v = [load_w(2, 0, 8, 11), load_w(2, 8, 16, 12)]
    wou = wo_hbm.bitcast(u32)
    c_o = [start(wou.at[:, pl.ds(n * 128, 128)], wobuf.at[n], 7) for n in range(DM // 128)]
    c_o.append(start(mem_hbm, membuf, 7))
    c_o.append(start(x_hbm.at[pl.ds(0, X1)], xbuf.at[pl.ds(0, X1)], 7))

    _wait('wc_w', c_w + c_q[1])
    _loop('preB', 4, 8, lambda u, _: pre(u, True))

    def mid_waits(i):
        wait_if(i == 10, c_q[3])
        wait_if(i == 22, c_k[0])
    _wait('wc_q2', c_q[2])
    _loop('mid', 8, H + NK, mid, 1, mid_waits)
    _wait('wc_inv', c_inv + c_k[1])

    def inv(m, _):
        zs = []
        for p in range(2):
            rhs = jnp.concatenate([jnp.concatenate([zbuf[t, :, 2 * m + p, c].reshape(N1, 128) for c in range(2)], axis=0)
                                   for t in range(5)], axis=1).astype(bf16)
            zs.append(jnp.dot(gibuf[2 * m + p], rhs, preferred_element_type=f32))
        ab = []
        for t in range(4):
            ln = slice(t * 128, (t + 1) * 128)
            re = [z[:N1, ln] for z in zs]
            im = [jnp.where(lane0, z[:N1, 512:], z[N1:, ln]) if t == 0 else z[N1:, ln] for z in zs]
            lhs = jnp.concatenate([jnp.concatenate(re, axis=0), jnp.concatenate(im, axis=0)], axis=1)
            v = jnp.dot(lhs.astype(bf16), fdibuf[t], preferred_element_type=f32)
            ab.append((v[:, :128], v[:, 128:]))
        (p_, q_), (a1, b1), (a2, b2), (a3, b3) = ab
        u0, u2, u4, u6 = p_ + a2, p_ - a2, q_ + b2, q_ - b2
        u1, u3, d, e = a1 + a3, b1 + b3, (a1 - a3) * rt, (b1 - b3) * rt
        u5, u7 = e + d, e - d
        ys = (u0 + u1, u4 + u5, u2 + u3, u6 + u7, u0 - u1, u4 - u5, u2 - u3, u6 - u7)
        for a in range(8):
            y = pltpu.bitcast(ys[a].astype(bf16).astype(f32), u32)
            bxbuf[m, :, a * 128:(a + 1) * 128] = (y[:N1] >> 16) | y[N1:]
        relayout(NPAIR + 9 + 2 * m)
        relayout(NPAIR + 10 + 2 * m)
        return 0

    def inv_waits(i):
        wait_if(i == 3, c_v[0])
        wait_if(i == 7, c_v[1])
    _loop('inv', 0, N2 // 2, inv, UI, inv_waits)
    outu = out_hbm.bitcast(u32)

    c_x = start(x_hbm.at[pl.ds(X1, NSEG - X1)], xbuf.at[pl.ds(X1, NSEG - X1)], 8)
    c_out = [start(bxbuf.at[m], outu.at[:, m, pl.ds(DM, DM)], 0) for m in range(N2 // 2)]
    _wait('wc_o', c_o)

    hbuf[0:M, :] = membuf[...].astype(f32)
    row = lax.broadcasted_iota(jnp.int32, (L, 128), 0)
    col = lax.broadcasted_iota(jnp.int32, (L, 128), 1)
    mask = (col < L) & ((row < M) | (row >= col))
    scale = DH ** -0.5

    def ycopy(s):
        return pltpu.make_async_copy(ybuf.at[s], out_hbm.at[s, :, pl.ds(0, DM)], sems.at[1])

    def step(s, _):
        hbuf[M:L, :] = xbuf[s].astype(f32)
        st = {}
        acc = [None] * (DM // 128)

        def proj(h):
            hv = hbuf[...]
            rows = pl.ds(pl.multiple_of(s % (NSEG // 2) * NP, NP), NP)
            if h < NK:
                k = jnp.dot(hv[:L - NP], getw(NPAIR + h // 2, h % 2), preferred_element_type=f32)
                k = jnp.concatenate([k, qkbuf[NPAIR + h // 2, h % 2, s // (NSEG // 2), rows, :]], axis=0)
            else:
                k = jnp.dot(hv, getw(NPAIR + h // 2, h % 2), preferred_element_type=f32)
            q = jnp.dot(hv[:L - NP], getw(h // 2, h % 2), preferred_element_type=f32)
            q = jnp.concatenate([q, qkbuf[h // 2, h % 2, s // (NSEG // 2), rows, :]], axis=0)
            v = jnp.dot(hv, getw(2 * NPAIR + h // 2, h % 2), preferred_element_type=f32)
            zpad = jnp.zeros((128 - L, DH), f32)
            st[h] = (q, jnp.concatenate([k, zpad], axis=0).astype(bf16),
                     jnp.concatenate([v, zpad], axis=0).astype(bf16))

        def qk(h):
            q, kp, vp = st[h]
            st[h] = (lax.dot_general(q, kp, (((1,), (1,)), ((), ())), preferred_element_type=f32), vp)

        def soft(h):
            sc, vp = st[h]
            sc = jnp.where(mask, sc, -1e30)
            e = jnp.exp2((sc - jnp.max(sc, axis=1, keepdims=True)) * (scale * math.log2(math.e)))
            l = jnp.sum(e, axis=1, keepdims=True)
            r = pl.reciprocal(l, approx=True)
            st[h] = (e, r * (2.0 - l * r), vp)

        def pv(h):
            e, r, vp = st.pop(h)
            obuf[:, h * DH:(h + 1) * DH] = jnp.dot(e, vp, preferred_element_type=f32) * r

        def out(h0, h1, n):
            w = pltpu.bitcast(wobuf[n, h0 * DH // 2:h1 * DH // 2, :], bf16)
            y = jnp.dot(obuf[:, h0 * DH:h1 * DH], w, preferred_element_type=f32)
            acc[n] = y if h0 == 0 else acc[n] + y
            if h1 == H:
                hbuf[0:M, n * 128:(n + 1) * 128] = acc[n][0:M].astype(bf16).astype(f32)
                ybuf[s, :, n * 128:(n + 1) * 128] = acc[n][M:L].astype(bf16)

        fns = dict(proj=proj, qk=qk, soft=soft, pv=pv, out=out)
        for name, *a in _schedule():
            fns[name](*a)
        ycopy(s).start()
        return 0

    def phase(ph, _):
        @pl.when(ph == 1)
        def _():
            c_x.wait()

        def steps(i, _):
            for j in range(US):
                step(i * US + j, 0)
            return 0
        lax.fori_loop(ph * (X1 // US), (X1 + ph * (NSEG - X1)) // US, steps, 0)
        return 0
    _loop('step', 0, 2, phase)
    _wait('wc_out', c_out)
    pltpu.make_async_copy(ybuf, ybuf, sems.at[1]).wait()


@jax.jit
def pallas_concat_heads__memory_aug_recurrent_mem_tr__spectral_gfnet__prompt_kernel(
        A_x, A_mem0, A_Wq, A_Wk, A_Wv, A_Wo, A_seg_len, B_x, B_w_r, B_w_i):
    del A_seg_len
    fd, fdi, g, gi = _consts()
    rw = lambda w: w.reshape(DM // 16, 16, H, DH)
    hbm = pl.BlockSpec(memory_space=pltpu.HBM)
    vm = pltpu.VMEM
    args = (A_x.reshape(NSEG, SEG, DM), A_mem0.reshape(M, DM), rw(A_Wq), rw(A_Wk), rw(A_Wv),
            A_Wo.reshape(H * DH, DM), B_x.reshape(N1, N2, DM), B_w_r.T, B_w_i.T, fd, fdi, g, gi)
    out = pl.pallas_call(
        _kernel,
        out_shape=jax.ShapeDtypeStruct((N1, N2, 2 * DM), bf16),
        in_specs=[hbm] * 13,
        out_specs=hbm,
        scratch_shapes=[
            vm((NSEG, SEG, DM), bf16), vm((M, DM), bf16),
            vm((3 * NPAIR + 9, DM // 16, 16, DH), u32), vm((DM // 128, H * DH // 2, 128), u32),
            vm((L, DM), f32), vm((L, H * DH), f32), vm((NSEG, SEG, DM), bf16),
            vm((N2 // 2, N1, DM), u32), vm((2, S // 128, DM // 4, 128), u32), vm((2, 1, S), bf16), vm((5, 8, N2, 8, 128), u32),
            vm((4, 256, 256), bf16), vm((4, 256, 256), bf16), vm((N2, 128, 128), bf16), vm((N2, 128, 128), bf16),
            vm((5, 8, N2, 2, 8, 128), f32), vm((NSEG, NP, DM), bf16), vm((2, NSEG * NP // 2, DM), f32), vm(((H + NK) // 2, 2, 2, NSEG * NP // 2, DH), f32),
            pltpu.SemaphoreType.DMA((16,))],
        compiler_params=pltpu.CompilerParams(vmem_limit_bytes=110 * 1024 * 1024),
    )(*[pltpu.with_memory_space_constraint(jnp.asarray(t), pltpu.HBM) for t in args])
    return out.reshape(1, S, 2 * DM)
```

```python
import functools
import math
import numpy as np
import jax
import jax.numpy as jnp
from jax import lax
from jax.experimental import pallas as pl
from jax.experimental.pallas import tpu as pltpu

S, DM, H, DH, M, SEG = 2048, 1024, 32, 128, 8, 32
L = M + SEG
NSEG = S // SEG
N1, N2 = 64, 32
NPAIR = H // 2
NP, NK = 8, 16
PSTEP, DIST = 64, 2
US, X1 = 4, 4
f32, bf16, u32 = jnp.float32, jnp.bfloat16, jnp.uint32


def _schedule():
    ev = []
    for h in range(H):
        ev.append(("proj", h))
        g, r = h // 4 - 1, h % 4
        if g >= 0:
            if r == 0:
                ev += [("qk", 4 * g + i) for i in range(4)]
            elif r == 3:
                ev += [("pv", 4 * g + i) for i in range(4)]
            else:
                ev += [("soft", 4 * g + 2 * r - 2), ("soft", 4 * g + 2 * r - 1)]
    o = lambda h0, h1, ns: [("out", h0, h1, n) for n in ns]
    ev += o(0, 8, (0, 1)) + [("qk", h) for h in range(28, 32)] + o(0, 8, (2, 3))
    for i in range(4):
        ev += [("soft", 28 + i)] + o(0, 8, (4 + i,))
    ev += o(8, 16, range(4)) + [("pv", h) for h in range(28, 32)] + o(8, 16, range(4, 8)) + o(16, 32, range(8))
    return ev


_CLS = ((0, 4), (1, 7), (2, 6), (3, 5))
_BETA = {0: 1, 4: -1, 1: -1j, 7: 1j, 2: -1j, 6: 1j, 3: 1j, 5: -1j}


def _consts():
    b = np.arange(128)[:, None]
    fd = np.zeros((4, 256, 256))
    fdi = np.zeros((4, 256, 256))
    for t, cls in enumerate(_CLS):
        k = np.concatenate([c + 8 * np.arange(64) for c in cls])[None, :]
        beta = np.concatenate([np.full(64, _BETA[c], np.complex128) for c in cls])[None, :]
        e = np.exp(-2j * np.pi * ((b * k) % DM) / DM)
        m = np.concatenate([e, beta * e], axis=0)
        re, im = m.real.copy(), m.imag.copy()
        wt = np.full((256,), 2.0)
        if t == 0:
            im[:, 0] = np.tile(np.cos(np.pi * b[:, 0]), 2)
            wt[0] = wt[128] = 1.0
        fd[t] = np.concatenate([re, im], axis=1)
        fdi[t] = fd[t].T * wt[:, None] / (S * DM)
    n2 = np.arange(N2)[:, None, None]
    k1 = np.arange(N1)[None, :, None]
    n1 = np.arange(N1)[None, None, :]
    a = 2 * np.pi * ((k1 * (N2 * n1 + n2)) % S) / S
    c, s = np.cos(a), -np.sin(a)
    g = np.concatenate([np.concatenate([c, -s], axis=2), np.concatenate([s, c], axis=2)], axis=1)
    gi = np.transpose(g, (0, 2, 1))
    cast = lambda t: np.ascontiguousarray(t).astype(np.float32).astype(jnp.bfloat16)
    return cast(fd), cast(fdi), cast(g), cast(gi)


def _tw(z, k, n):
    k %= n
    zr, zi = z
    if k == 0:
        return z
    if 4 * k == n:
        return (zi, -zr)
    if 2 * k == n:
        return (-zr, -zi)
    if 4 * k == 3 * n:
        return (-zi, zr)
    c, s = math.cos(2 * math.pi * k / n), -math.sin(2 * math.pi * k / n)
    if (8 * k) % n == 0:
        r = math.sqrt(0.5)
        if 8 * k == n:
            return ((zr + zi) * r, (zi - zr) * r)
        if 8 * k == 3 * n:
            return ((zi - zr) * r, (zr + zi) * (-r))
    return (zr * c - zi * s, zr * s + zi * c)


def _fft(x):
    n = len(x)
    if n == 1:
        return x
    if n == 2:
        (ar, ai), (br, bi) = x
        return [(ar + br, ai + bi), (ar - br, ai - bi)]
    e, o1, o3 = _fft(x[0::2]), _fft(x[1::4]), _fft(x[3::4])
    out = [None] * n
    q = n // 4
    for k in range(q):
        t1, t3 = _tw(o1[k], k, n), _tw(o3[k], 3 * k, n)
        sr, si = t1[0] + t3[0], t1[1] + t3[1]
        dr, di = t1[0] - t3[0], t1[1] - t3[1]
        out[k] = (e[k][0] + sr, e[k][1] + si)
        out[k + 2 * q] = (e[k][0] - sr, e[k][1] - si)
        out[k + q] = (e[k + q][0] + di, e[k + q][1] - dr)
        out[k + 3 * q] = (e[k + q][0] - di, e[k + q][1] + dr)
    return out


def _ifft(x):
    return [(b, a) for a, b in _fft([(b, a) for a, b in x])]


def _loop(lo, hi, fn):
    def body(i, c):
        fn(i)
        return c
    lax.fori_loop(lo, hi, body, 0)


def _wait(cs):
    for c in cs:
        c.wait()


def _lo(w):
    return pltpu.bitcast(w << 16, f32)


def _hi(w):
    return pltpu.bitcast(w & jnp.uint32(0xFFFF0000), f32)


def _kernel(x_hbm, mem_hbm, wq_hbm, wk_hbm, wv_hbm, wo_hbm, bx_hbm, wr_hbm, wi_hbm,
            fd_hbm, fdi_hbm, g_hbm, gi_hbm, out_hbm,
            xbuf, membuf, wbuf, wobuf, hbuf, obuf, ybuf,
            bxbuf, wtbuf, wnbuf, wpbuf, fdbuf, fdibuf, gbuf, gibuf, zbuf, rbuf, lbuf, xqbuf, xfbuf, qkbuf, sems):
    def start(src, dst, i):
        c = pltpu.make_async_copy(src, dst, sems.at[i])
        c.start()
        return c

    bxu = bx_hbm.bitcast(u32)

    def load_f(m0, m1, sem):
        gs = pl.ds(2 * m0, 2 * (m1 - m0))
        return ([start(g_hbm.at[gs], gbuf.at[gs], sem)]
                + [start(bxu.at[:, m, :], bxbuf.at[m], sem) for m in range(m0, m1)])

    c_f = [start(fd_hbm, fdbuf, 0)] + load_f(0, 2, 0)
    c_f2 = [load_f(2, 4, 1), load_f(4, 8, 13), load_f(8, 16, 14)]
    def load_w(t, j0, j1, sem):
        wu = (wq_hbm, wk_hbm, wv_hbm)[t].bitcast(u32)
        return [start(wu.at[:, :, j, :], wbuf.at[t * NPAIR + j], sem) for j in range(j0, j1)]

    def getw(u, p):
        w = wbuf[u, :, pl.ds(p * 8, 8), :]
        return pltpu.bitcast(w.reshape(DM // 2, DH), bf16)

    def relayout(u, half, pace=None):
        for i in range(32):
            g = 32 * half + i
            a = wbuf[u, g, pl.ds(0, 8, stride=2), :]
            b = wbuf[u, g, pl.ds(1, 8, stride=2), :]
            if pace is not None:
                a = jnp.where(u < 0, pltpu.bitcast(pace[i], u32), a)
            wbuf[u, g, 0:8, :] = (a & jnp.uint32(0xFFFF)) | (b << 16)
            wbuf[u, g, 8:16, :] = (a >> 16) | (b & jnp.uint32(0xFFFF0000))

    def wait_if(cond, cs):
        @pl.when(cond)
        def _():
            for c in cs:
                c.wait()

    lane0 = lax.broadcasted_iota(jnp.int32, (N1, 128), 1) == 0
    rt = math.sqrt(0.5)

    def fwd_d(m):
        w = bxbuf[m]
        xs = [jnp.concatenate([_lo(w[:, a * 128:(a + 1) * 128]), _hi(w[:, a * 128:(a + 1) * 128])], axis=0)
              for a in range(8)]
        u0, u1, u2, u3 = xs[0] + xs[4], xs[0] - xs[4], xs[2] + xs[6], xs[2] - xs[6]
        u4, u5, u6, u7 = xs[1] + xs[5], xs[1] - xs[5], xs[3] + xs[7], xs[3] - xs[7]
        d, e = (u5 - u7) * rt, (u5 + u7) * rt
        ab = ((u0 + u2, u4 + u6), (u1 + d, u3 + e), (u0 - u2, u4 - u6), (u1 - d, u3 - e))
        z = [jnp.dot(jnp.concatenate(ab[t], axis=1).astype(bf16), fdbuf[t], preferred_element_type=f32)
             for t in range(4)]
        for p in range(2):
            rows = slice(p * N1, (p + 1) * N1)
            zi0 = z[0][rows, 128:]
            top = [z[t][rows, :128] for t in range(4)] + [jnp.where(lane0, zi0, 0.0)]
            bot = [jnp.where(lane0, 0.0, zi0)] + [z[t][rows, 128:] for t in range(1, 4)] + [jnp.zeros((N1, 128), f32)]
            rhs = jnp.concatenate([jnp.concatenate(top, axis=1), jnp.concatenate(bot, axis=1)], axis=0)
            rbuf[p] = rhs.astype(bf16)

    def fwd_s(m):
        for p in range(2):
            y = jnp.dot(gbuf[2 * m + p], rbuf[p], preferred_element_type=f32)
            for t in range(5):
                for c in range(2):
                    zbuf[t, :, 2 * m + p, c] = y[c * N1:(c + 1) * N1, t * 128:(t + 1) * 128].reshape(8, 8, 128)

    def fwd(m):
        for c, m0 in zip(c_f2, (2, 4, 8)):
            wait_if(m == m0, c)
        fwd_s(m - 1)
        fwd_d(m)

    def permute_w(jt):
        def put(i, v):
            v = v.T
            for c in range(2):
                wpbuf[i, :, 2 * jt + c] = v[c * N1:(c + 1) * N1].reshape(8, 8, 128)
        ln = pl.ds(pl.multiple_of(jt * 128, 128), 128)
        for i in range(2):
            p = [wtbuf[i, jt, pl.ds(c, 64, stride=4), :] for c in range(4)]
            lo, hi = jnp.uint32(0xFFFF), jnp.uint32(0xFFFF0000)
            put(2 * i, jnp.concatenate([p[0], (p[2] & lo) | (p[3] & hi)], axis=0))
            put(2 * i + 1, jnp.concatenate([p[1], (p[3] & lo) | (p[2] & hi)], axis=0))
        nr = pltpu.bitcast(wnbuf[0, :, ln].astype(f32), u32)
        ni = pltpu.bitcast(wnbuf[1, :, ln].astype(f32), u32)
        put(4, jnp.broadcast_to((nr >> 16) | ni, (128, 128)))

    c_q = [[start(x_hbm.at[:, pl.ds(SEG - NP, NP), :], xqbuf, 4)] + load_w(0, 0, 3, 4)]
    c_w = []
    for i, w in enumerate((wr_hbm, wi_hbm)):
        wu = w.at[pl.ds(0, DM // 2), :].bitcast(u32)
        c_w += [start(wu.at[:, pl.ds(j * 128, 128)], wtbuf.at[i, j], 2) for j in range(S // 128)]
        c_w.append(start(w.at[pl.ds(DM // 2, 1), :], wnbuf.at[i], 2))

    _wait(c_f)
    fwd_d(0)
    _loop(1, N2 // 2, fwd)
    fwd_s(N2 // 2 - 1)
    c_q += [load_w(0, 3, 5, 5), load_w(0, 5, 10, 6), load_w(0, 10, 16, 15)]
    c_inv = [start(fdi_hbm, fdibuf, 3), start(gi_hbm, gibuf, 3)]
    c_k = [load_w(1, 0, 9, 9), load_w(1, 9, 16, 10)]
    def mid_pieces(g, t, res):
        def lds(ns):
            z = [(zbuf[t, g, n, 0], zbuf[t, g, n, 1]) for n in ns]
            if len(res) >= DIST:
                z[0] = (jnp.where(t < 0, res[-DIST], z[0][0]), z[0][1])
                z[1] = (z[1][0], jnp.where(t < 0, res[-DIST], z[1][1]))
            return z
        nyq = t // 4
        ir, ii = t // 2 + 2 * nyq, t // 2 + 2
        sr = (16 * (1 - t % 2)).astype(u32)
        si = (16 * (1 - t % 2 - nyq)).astype(u32)
        half = lambda w, sh: pltpu.bitcast((w << sh) & jnp.uint32(0xFFFF0000), f32)

        def st(n, z):
            zbuf[t, g, n, 0] = z[0]
            zbuf[t, g, n, 1] = z[1]

        def p1(b):
            y = _fft(lds([4 * a + b for a in range(8)]))
            for ka in range(8):
                st(4 * ka + b, _tw(y[ka], b * ka, N2))

        def p2(ka):
            y = _fft(lds([4 * ka + b for b in range(4)]))
            for kb in range(4):
                wr, wi = half(wpbuf[ir, g, ka + 8 * kb], sr), half(wpbuf[ii, g, ka + 8 * kb], si)
                yr, yi = y[kb]
                y[kb] = (yr * wr - yi * wi, yr * wi + yi * wr)
            y = _ifft(y)
            for b in range(4):
                st(4 * ka + b, _tw(y[b], -b * ka, N2))

        def p3(b):
            y = _ifft(lds([4 * ka + b for ka in range(8)]))
            for a in range(8):
                st(4 * a + b, y[a])

        P = functools.partial
        return [P(p1, b) for b in range(4)] + [P(p2, k) for k in range(8)] + [P(p3, b) for b in range(4)]

    def pre_pieces(u, step, res):
        def piece(p, r):
            y = jnp.dot(xfbuf[u % 2, r:r + step, :], getw(u // 2, p), preferred_element_type=f32)
            res.append(y[0:8])
            qkbuf[u // 2, p, u % 2, r:r + step, :] = y
        return [functools.partial(piece, p, r) for p in range(2) for r in range(0, NSEG * NP // 2, step)]

    def mid(u):
        wait_if(u == 18, c_q[3])
        wait_if(u == 30, c_k[0])
        res = []
        mp = mid_pieces((u - 8) // 5, (u - 8) % 5, res)
        pp = pre_pieces(u, PSTEP, res)
        k = len(mp) // len(pp)
        for c, p in enumerate(pp):
            p()
            for f in mp[c * k:(c + 1) * k]:
                f()
        relayout(u // 2 + 1, u % 2)

    def pre(u, with_w):
        for p in pre_pieces(u, 256, []):
            p()
        if with_w:
            for j in range(4):
                permute_w(4 * (u - 4) + j)
        relayout(u // 2 + 1, u % 2)

    _wait(c_q[0])
    xfbuf[...] = xqbuf[...].astype(f32).reshape(2, NSEG * NP // 2, DM)
    relayout(0, 0)
    relayout(0, 1)
    _loop(0, 4, lambda u: pre(u, False))
    c_v = [load_w(2, 0, 8, 11), load_w(2, 8, 16, 12)]
    wou = wo_hbm.bitcast(u32)
    c_o = [start(wou.at[:, pl.ds(n * 128, 128)], wobuf.at[n], 7) for n in range(DM // 128)]
    c_o.append(start(mem_hbm, membuf, 7))
    c_o.append(start(x_hbm.at[pl.ds(0, X1)], xbuf.at[pl.ds(0, X1)], 7))

    _wait(c_w + c_q[1])
    _loop(4, 8, lambda u: pre(u, True))

    _wait(c_q[2])
    _loop(8, H + NK, mid)
    _wait(c_inv + c_k[1])

    def inv_s(m):
        zs = []
        for p in range(2):
            rhs = jnp.concatenate([jnp.concatenate([zbuf[t, :, 2 * m + p, c].reshape(N1, 128) for c in range(2)], axis=0)
                                   for t in range(5)], axis=1).astype(bf16)
            zs.append(jnp.dot(gibuf[2 * m + p], rhs, preferred_element_type=f32))
        for t in range(4):
            ln = slice(t * 128, (t + 1) * 128)
            re = [z[:N1, ln] for z in zs]
            im = [jnp.where(lane0, z[:N1, 512:], z[N1:, ln]) if t == 0 else z[N1:, ln] for z in zs]
            lhs = jnp.concatenate([jnp.concatenate(re, axis=0), jnp.concatenate(im, axis=0)], axis=1)
            lbuf[t] = lhs.astype(bf16)

    def inv(m, nxt):
        if nxt:
            wait_if(m == 4, c_v[0])
            wait_if(m == 10, c_v[1])
        ab = []
        for t in range(4):
            v = jnp.dot(lbuf[t], fdibuf[t], preferred_element_type=f32)
            ab.append((v[:, :128], v[:, 128:]))
        if nxt:
            for c in range(3):
                q = 3 * m + c
                relayout((H + NK) // 2 + 1 + q // 2, q % 2,
                         [ab[c][i % 2][8 * (i // 2):8 * (i // 2) + 8] for i in range(32)])
            inv_s(m + 1)
        (p_, q_), (a1, b1), (a2, b2), (a3, b3) = ab
        u0, u2, u4, u6 = p_ + a2, p_ - a2, q_ + b2, q_ - b2
        u1, u3, d, e = a1 + a3, b1 + b3, (a1 - a3) * rt, (b1 - b3) * rt
        u5, u7 = e + d, e - d
        ys = (u0 + u1, u4 + u5, u2 + u3, u6 + u7, u0 - u1, u4 - u5, u2 - u3, u6 - u7)
        for a in range(8):
            y = pltpu.bitcast(ys[a].astype(bf16).astype(f32), u32)
            bxbuf[m, :, a * 128:(a + 1) * 128] = (y[:N1] >> 16) | y[N1:]

    inv_s(0)
    _loop(0, N2 // 2 - 1, lambda m: inv(m, True))
    inv(N2 // 2 - 1, False)
    relayout(3 * NPAIR - 1, 1)
    outu = out_hbm.bitcast(u32)

    c_x = start(x_hbm.at[pl.ds(X1, NSEG - X1)], xbuf.at[pl.ds(X1, NSEG - X1)], 8)
    c_out = [start(bxbuf.at[m], outu.at[:, m, pl.ds(DM, DM)], 0) for m in range(N2 // 2)]
    _wait(c_o)

    hbuf[0:M, :] = membuf[...].astype(f32)
    row = lax.broadcasted_iota(jnp.int32, (L, 128), 0)
    col = lax.broadcasted_iota(jnp.int32, (L, 128), 1)
    mask = (col < L) & ((row < M) | (row >= col))
    scale = DH ** -0.5
    fill = jnp.where(col < L, -1e9 / scale, -jnp.inf)

    def ycopy(s):
        return pltpu.make_async_copy(ybuf.at[s], out_hbm.at[s, :, pl.ds(0, DM)], sems.at[1])

    def step(s):
        hbuf[M:L, :] = xbuf[s].astype(f32)
        st = {}
        acc = [None] * (DM // 128)

        def proj(h):
            hv = hbuf[...]
            rows = pl.ds(pl.multiple_of(s % (NSEG // 2) * NP, NP), NP)
            if h < NK:
                k = jnp.dot(hv[:L - NP], getw(NPAIR + h // 2, h % 2), preferred_element_type=f32)
                k = jnp.concatenate([k, qkbuf[NPAIR + h // 2, h % 2, s // (NSEG // 2), rows, :]], axis=0)
            else:
                k = jnp.dot(hv, getw(NPAIR + h // 2, h % 2), preferred_element_type=f32)
            q = jnp.dot(hv[:L - NP], getw(h // 2, h % 2), preferred_element_type=f32)
            q = jnp.concatenate([q, qkbuf[h // 2, h % 2, s // (NSEG // 2), rows, :]], axis=0)
            v = jnp.dot(hv, getw(2 * NPAIR + h // 2, h % 2), preferred_element_type=f32)
            zpad = jnp.zeros((128 - L, DH), f32)
            st[h] = (q, jnp.concatenate([k, zpad], axis=0).astype(bf16),
                     jnp.concatenate([v, zpad], axis=0).astype(bf16))

        def qk(h):
            q, kp, vp = st[h]
            st[h] = (lax.dot_general(q, kp, (((1,), (1,)), ((), ())), preferred_element_type=f32), vp)

        def soft(h):
            sc, vp = st[h]
            sc = jnp.where(mask, sc, fill)
            e = jnp.exp2((sc - jnp.max(sc, axis=1, keepdims=True)) * (scale * math.log2(math.e)))
            l = jnp.sum(e, axis=1, keepdims=True)
            r = pl.reciprocal(l, approx=True)
            st[h] = (e, r * (2.0 - l * r), vp)

        def pv(h):
            e, r, vp = st.pop(h)
            obuf[:, h * DH:(h + 1) * DH] = jnp.dot(e, vp, preferred_element_type=f32) * r

        def out(h0, h1, n):
            w = pltpu.bitcast(wobuf[n, h0 * DH // 2:h1 * DH // 2, :], bf16)
            y = jnp.dot(obuf[:, h0 * DH:h1 * DH], w, preferred_element_type=f32)
            acc[n] = y if h0 == 0 else acc[n] + y
            if h1 == H:
                hbuf[0:M, n * 128:(n + 1) * 128] = acc[n][0:M].astype(bf16).astype(f32)
                ybuf[s, :, n * 128:(n + 1) * 128] = acc[n][M:L].astype(bf16)

        fns = dict(proj=proj, qk=qk, soft=soft, pv=pv, out=out)
        for name, *a in _schedule():
            fns[name](*a)
        ycopy(s).start()

    def steps(i):
        for j in range(US):
            step(i * US + j)

    def phase(ph):
        wait_if(ph == 1, [c_x])
        _loop(ph * (X1 // US), (X1 + ph * (NSEG - X1)) // US, steps)

    _loop(0, 2, phase)
    _wait(c_out)
    _loop(0, NSEG, lambda s: ycopy(s).wait())


@jax.jit
def pallas_concat_heads__memory_aug_recurrent_mem_tr__spectral_gfnet__prompt_kernel(
        A_x, A_mem0, A_Wq, A_Wk, A_Wv, A_Wo, A_seg_len, B_x, B_w_r, B_w_i):
    del A_seg_len
    fd, fdi, g, gi = _consts()
    rw = lambda w: w.reshape(DM // 16, 16, H, DH)
    hbm = pl.BlockSpec(memory_space=pltpu.HBM)
    vm = pltpu.VMEM
    args = (A_x.reshape(NSEG, SEG, DM), A_mem0.reshape(M, DM), rw(A_Wq), rw(A_Wk), rw(A_Wv),
            A_Wo.reshape(H * DH, DM), B_x.reshape(N1, N2, DM), B_w_r.T, B_w_i.T, fd, fdi, g, gi)
    out = pl.pallas_call(
        _kernel,
        out_shape=jax.ShapeDtypeStruct((N1, N2, 2 * DM), bf16),
        in_specs=[hbm] * 13,
        out_specs=hbm,
        scratch_shapes=[
            vm((NSEG, SEG, DM), bf16), vm((M, DM), bf16),
            vm((3 * NPAIR, DM // 16, 16, DH), u32), vm((DM // 128, H * DH // 2, 128), u32),
            vm((L, DM), f32), vm((L, H * DH), f32), vm((NSEG, SEG, DM), bf16),
            vm((N2 // 2, N1, DM), u32), vm((2, S // 128, DM // 4, 128), u32), vm((2, 1, S), bf16), vm((5, 8, N2, 8, 128), u32),
            vm((4, 256, 256), bf16), vm((4, 256, 256), bf16), vm((N2, 128, 128), bf16), vm((N2, 128, 128), bf16),
            vm((5, 8, N2, 2, 8, 128), f32), vm((2, 128, 640), bf16), vm((4, 128, 256), bf16), vm((NSEG, NP, DM), bf16), vm((2, NSEG * NP // 2, DM), f32), vm(((H + NK) // 2, 2, 2, NSEG * NP // 2, DH), f32),
            pltpu.SemaphoreType.DMA((16,))],
        compiler_params=pltpu.CompilerParams(vmem_limit_bytes=110 * 1024 * 1024),
    )(*[pltpu.with_memory_space_constraint(jnp.asarray(t), pltpu.HBM) for t in args])
    return out.reshape(1, S, 2 * DM)
```

```python
import functools
import math
import numpy as np
import jax
import jax.numpy as jnp
from jax import lax
from jax.experimental import pallas as pl
from jax.experimental.pallas import tpu as pltpu

S, DM, H, DH, M, SEG = 2048, 1024, 32, 128, 8, 32
L = M + SEG
NSEG = S // SEG
N1, N2 = 64, 32
NPAIR = H // 2
NP, NK = 8, 16
PSTEP, DIST = 64, 2
US, X1 = 4, 4
f32, bf16, u32 = jnp.float32, jnp.bfloat16, jnp.uint32


def _schedule():
    ev = []
    for h in range(H):
        ev.append(("proj", h))
        g, r = h // 4 - 1, h % 4
        if g >= 0:
            if r == 0:
                ev += [("qk", 4 * g + i) for i in range(4)]
            elif r == 3:
                ev += [("pv", 4 * g + i) for i in range(4)]
            else:
                ev += [("soft", 4 * g + 2 * r - 2), ("soft", 4 * g + 2 * r - 1)]
    o = lambda h0, h1, ns: [("out", h0, h1, n) for n in ns]
    ev += o(0, 8, (0, 1)) + [("qk", h) for h in range(28, 32)] + o(0, 8, (2, 3))
    for i in range(4):
        ev += [("soft", 28 + i)] + o(0, 8, (4 + i,))
    ev += o(8, 16, range(4)) + [("pv", h) for h in range(28, 32)] + o(8, 16, range(4, 8)) + o(16, 32, range(8))
    return ev


_CLS = ((0, 4), (1, 7), (2, 6), (3, 5))
_BETA = {0: 1, 4: -1, 1: -1j, 7: 1j, 2: -1j, 6: 1j, 3: 1j, 5: -1j}


def _consts():
    b = np.arange(128)[:, None]
    fd = np.zeros((4, 256, 256))
    fdi = np.zeros((4, 256, 256))
    for t, cls in enumerate(_CLS):
        k = np.concatenate([c + 8 * np.arange(64) for c in cls])[None, :]
        beta = np.concatenate([np.full(64, _BETA[c], np.complex128) for c in cls])[None, :]
        e = np.exp(-2j * np.pi * ((b * k) % DM) / DM)
        m = np.concatenate([e, beta * e], axis=0)
        re, im = m.real.copy(), m.imag.copy()
        wt = np.full((256,), 2.0)
        if t == 0:
            im[:, 0] = np.tile(np.cos(np.pi * b[:, 0]), 2)
            wt[0] = wt[128] = 1.0
        fd[t] = np.concatenate([re, im], axis=1)
        fdi[t] = fd[t].T * wt[:, None] / (S * DM)
    n2 = np.arange(N2)[:, None, None]
    k1 = np.arange(N1)[None, :, None]
    n1 = np.arange(N1)[None, None, :]
    a = 2 * np.pi * ((k1 * (N2 * n1 + n2)) % S) / S
    c, s = np.cos(a), -np.sin(a)
    g = np.concatenate([np.concatenate([c, -s], axis=2), np.concatenate([s, c], axis=2)], axis=1)
    gi = np.transpose(g, (0, 2, 1))
    cast = lambda t: np.ascontiguousarray(t).astype(np.float32).astype(jnp.bfloat16)
    return cast(fd), cast(fdi), cast(g), cast(gi)


def _tw(z, k, n):
    k %= n
    zr, zi = z
    if k == 0:
        return z
    if 4 * k == n:
        return (zi, -zr)
    if 2 * k == n:
        return (-zr, -zi)
    if 4 * k == 3 * n:
        return (-zi, zr)
    c, s = math.cos(2 * math.pi * k / n), -math.sin(2 * math.pi * k / n)
    if (8 * k) % n == 0:
        r = math.sqrt(0.5)
        if 8 * k == n:
            return ((zr + zi) * r, (zi - zr) * r)
        if 8 * k == 3 * n:
            return ((zi - zr) * r, (zr + zi) * (-r))
    return (zr * c - zi * s, zr * s + zi * c)


def _fft(x):
    n = len(x)
    if n == 1:
        return x
    if n == 2:
        (ar, ai), (br, bi) = x
        return [(ar + br, ai + bi), (ar - br, ai - bi)]
    e, o1, o3 = _fft(x[0::2]), _fft(x[1::4]), _fft(x[3::4])
    out = [None] * n
    q = n // 4
    for k in range(q):
        t1, t3 = _tw(o1[k], k, n), _tw(o3[k], 3 * k, n)
        sr, si = t1[0] + t3[0], t1[1] + t3[1]
        dr, di = t1[0] - t3[0], t1[1] - t3[1]
        out[k] = (e[k][0] + sr, e[k][1] + si)
        out[k + 2 * q] = (e[k][0] - sr, e[k][1] - si)
        out[k + q] = (e[k + q][0] + di, e[k + q][1] - dr)
        out[k + 3 * q] = (e[k + q][0] - di, e[k + q][1] + dr)
    return out


def _ifft(x):
    return [(b, a) for a, b in _fft([(b, a) for a, b in x])]


def _loop(lo, hi, fn):
    def body(i, c):
        fn(i)
        return c
    lax.fori_loop(lo, hi, body, 0)


def _wait(cs):
    for c in cs:
        c.wait()


def _lo(w):
    return pltpu.bitcast(w << 16, f32)


def _hi(w):
    return pltpu.bitcast(w & jnp.uint32(0xFFFF0000), f32)


def _kernel(x_hbm, mem_hbm, wq_hbm, wk_hbm, wv_hbm, wo_hbm, bx_hbm, wr_hbm, wi_hbm,
            fd_hbm, fdi_hbm, g_hbm, gi_hbm, out_hbm,
            xbuf, membuf, wbuf, wobuf, hbuf, obuf, ybuf,
            bxbuf, wtbuf, wnbuf, wpbuf, fdbuf, fdibuf, gbuf, gibuf, zbuf, rbuf, lbuf, xqbuf, xfbuf, qkbuf, sems):
    def start(src, dst, i):
        c = pltpu.make_async_copy(src, dst, sems.at[i])
        c.start()
        return c

    bxu = bx_hbm.bitcast(u32)

    def load_f(m0, m1, sem):
        gs = pl.ds(2 * m0, 2 * (m1 - m0))
        return ([start(g_hbm.at[gs], gbuf.at[gs], sem)]
                + [start(bxu.at[:, m, :], bxbuf.at[m], sem) for m in range(m0, m1)])

    c_f = [start(fd_hbm, fdbuf, 0)] + load_f(0, 2, 0)
    c_f2 = [load_f(2, 4, 1), load_f(4, 8, 13), load_f(8, 16, 14)]
    def load_w(t, j0, j1, sem):
        wu = (wq_hbm, wk_hbm, wv_hbm)[t].bitcast(u32)
        return [start(wu.at[:, :, j, :], wbuf.at[t * NPAIR + j], sem) for j in range(j0, j1)]

    def getw(u, p):
        w = wbuf[u, :, pl.ds(p * 8, 8), :]
        return pltpu.bitcast(w.reshape(DM // 2, DH), bf16)

    def relayout(u, half, pace=None):
        for i in range(32):
            g = 32 * half + i
            a = wbuf[u, g, pl.ds(0, 8, stride=2), :]
            b = wbuf[u, g, pl.ds(1, 8, stride=2), :]
            if pace is not None:
                a = jnp.where(u < 0, pltpu.bitcast(pace[i], u32), a)
            wbuf[u, g, 0:8, :] = (a & jnp.uint32(0xFFFF)) | (b << 16)
            wbuf[u, g, 8:16, :] = (a >> 16) | (b & jnp.uint32(0xFFFF0000))

    def wait_if(cond, cs):
        @pl.when(cond)
        def _():
            for c in cs:
                c.wait()

    lane0 = lax.broadcasted_iota(jnp.int32, (N1, 128), 1) == 0
    rt = math.sqrt(0.5)

    def fwd_d(m):
        w = bxbuf[m]
        xs = [jnp.concatenate([_lo(w[:, a * 128:(a + 1) * 128]), _hi(w[:, a * 128:(a + 1) * 128])], axis=0)
              for a in range(8)]
        u0, u1, u2, u3 = xs[0] + xs[4], xs[0] - xs[4], xs[2] + xs[6], xs[2] - xs[6]
        u4, u5, u6, u7 = xs[1] + xs[5], xs[1] - xs[5], xs[3] + xs[7], xs[3] - xs[7]
        d, e = (u5 - u7) * rt, (u5 + u7) * rt
        ab = ((u0 + u2, u4 + u6), (u1 + d, u3 + e), (u0 - u2, u4 - u6), (u1 - d, u3 - e))
        z = [jnp.dot(jnp.concatenate(ab[t], axis=1).astype(bf16), fdbuf[t], preferred_element_type=f32)
             for t in range(4)]
        for p in range(2):
            rows = slice(p * N1, (p + 1) * N1)
            zi0 = z[0][rows, 128:]
            top = [z[t][rows, :128] for t in range(4)] + [jnp.where(lane0, zi0, 0.0)]
            bot = [jnp.where(lane0, 0.0, zi0)] + [z[t][rows, 128:] for t in range(1, 4)] + [jnp.zeros((N1, 128), f32)]
            rhs = jnp.concatenate([jnp.concatenate(top, axis=1), jnp.concatenate(bot, axis=1)], axis=0)
            rbuf[p] = rhs.astype(bf16)

    def fwd_s(m):
        for p in range(2):
            y = jnp.dot(gbuf[2 * m + p], rbuf[p], preferred_element_type=f32)
            for t in range(5):
                for c in range(2):
                    zbuf[t, :, 2 * m + p, c] = y[c * N1:(c + 1) * N1, t * 128:(t + 1) * 128].reshape(8, 8, 128)

    def fwd(m):
        for c, m0 in zip(c_f2, (2, 4, 8)):
            wait_if(m == m0, c)
        fwd_s(m - 1)
        fwd_d(m)

    def permute_w(jt):
        def put(i, v):
            v = v.T
            for c in range(2):
                wpbuf[i, :, 2 * jt + c] = v[c * N1:(c + 1) * N1].reshape(8, 8, 128)
        ln = pl.ds(pl.multiple_of(jt * 128, 128), 128)
        for i in range(2):
            p = [wtbuf[i, jt, pl.ds(c, 64, stride=4), :] for c in range(4)]
            lo, hi = jnp.uint32(0xFFFF), jnp.uint32(0xFFFF0000)
            put(2 * i, jnp.concatenate([p[0], (p[2] & lo) | (p[3] & hi)], axis=0))
            put(2 * i + 1, jnp.concatenate([p[1], (p[3] & lo) | (p[2] & hi)], axis=0))
        nr = pltpu.bitcast(wnbuf[0, :, ln].astype(f32), u32)
        ni = pltpu.bitcast(wnbuf[1, :, ln].astype(f32), u32)
        put(4, jnp.broadcast_to((nr >> 16) | ni, (128, 128)))

    c_q = [[start(x_hbm.at[:, pl.ds(SEG - NP, NP), :], xqbuf, 4)] + load_w(0, 0, 3, 4)]
    c_w = []
    for i, w in enumerate((wr_hbm, wi_hbm)):
        wu = w.at[pl.ds(0, DM // 2), :].bitcast(u32)
        c_w += [start(wu.at[:, pl.ds(j * 128, 128)], wtbuf.at[i, j], 2) for j in range(S // 128)]
        c_w.append(start(w.at[pl.ds(DM // 2, 1), :], wnbuf.at[i], 2))

    _wait(c_f)
    fwd_d(0)
    _loop(1, N2 // 2, fwd)
    fwd_s(N2 // 2 - 1)
    c_q += [load_w(0, 3, 5, 5), load_w(0, 5, 10, 6), load_w(0, 10, 16, 15)]
    c_inv = [start(fdi_hbm, fdibuf, 3), start(gi_hbm, gibuf, 3)]
    c_k = [load_w(1, 0, 9, 9), load_w(1, 9, 16, 10)]
    def mid_pieces(g, t, res):
        def lds(ns):
            z = [(zbuf[t, g, n, 0], zbuf[t, g, n, 1]) for n in ns]
            if len(res) >= DIST:
                z[0] = (jnp.where(t < 0, res[-DIST], z[0][0]), z[0][1])
                z[1] = (z[1][0], jnp.where(t < 0, res[-DIST], z[1][1]))
            return z
        nyq = t // 4
        ir, ii = t // 2 + 2 * nyq, t // 2 + 2
        sr = (16 * (1 - t % 2)).astype(u32)
        si = (16 * (1 - t % 2 - nyq)).astype(u32)
        half = lambda w, sh: pltpu.bitcast((w << sh) & jnp.uint32(0xFFFF0000), f32)

        def st(n, z):
            zbuf[t, g, n, 0] = z[0]
            zbuf[t, g, n, 1] = z[1]

        def p1(b):
            y = _fft(lds([4 * a + b for a in range(8)]))
            for ka in range(8):
                st(4 * ka + b, _tw(y[ka], b * ka, N2))

        def p2(ka):
            y = _fft(lds([4 * ka + b for b in range(4)]))
            for kb in range(4):
                wr, wi = half(wpbuf[ir, g, ka + 8 * kb], sr), half(wpbuf[ii, g, ka + 8 * kb], si)
                yr, yi = y[kb]
                y[kb] = (yr * wr - yi * wi, yr * wi + yi * wr)
            y = _ifft(y)
            for b in range(4):
                st(4 * ka + b, _tw(y[b], -b * ka, N2))

        def p3(b):
            y = _ifft(lds([4 * ka + b for ka in range(8)]))
            for a in range(8):
                st(4 * a + b, y[a])

        P = functools.partial
        return [P(p1, b) for b in range(4)] + [P(p2, k) for k in range(8)] + [P(p3, b) for b in range(4)]

    def pre_pieces(u, step, res):
        def piece(p, r):
            y = jnp.dot(xfbuf[u % 2, r:r + step, :], getw(u // 2, p), preferred_element_type=f32)
            res.append(y[0:8])
            n = US * NP
            qkbuf[u // 2, p, u % 2, r // n:(r + step) // n] = y.reshape(step // n, n, DH)
        return [functools.partial(piece, p, r) for p in range(2) for r in range(0, NSEG * NP // 2, step)]

    def mid(u):
        wait_if(u == 18, c_q[3])
        wait_if(u == 30, c_k[0])
        res = []
        mp = mid_pieces((u - 8) // 5, (u - 8) % 5, res)
        pp = pre_pieces(u, PSTEP, res)
        k = len(mp) // len(pp)
        for c, p in enumerate(pp):
            p()
            for f in mp[c * k:(c + 1) * k]:
                f()
        relayout(u // 2 + 1, u % 2)

    def pre(u, with_w):
        for p in pre_pieces(u, 256, []):
            p()
        if with_w:
            for j in range(4):
                permute_w(4 * (u - 4) + j)
        relayout(u // 2 + 1, u % 2)

    _wait(c_q[0])
    xfbuf[...] = xqbuf[...].astype(f32).reshape(2, NSEG * NP // 2, DM)
    relayout(0, 0)
    relayout(0, 1)
    _loop(0, 4, lambda u: pre(u, False))
    c_v = [load_w(2, 0, 8, 11), load_w(2, 8, 16, 12)]
    wou = wo_hbm.bitcast(u32)
    c_o = [start(wou.at[:, pl.ds(n * 128, 128)], wobuf.at[n], 7) for n in range(DM // 128)]
    c_o.append(start(mem_hbm, membuf, 7))
    c_o.append(start(x_hbm.at[pl.ds(0, X1)], xbuf.at[pl.ds(0, X1)], 7))

    _wait(c_w + c_q[1])
    _loop(4, 8, lambda u: pre(u, True))

    _wait(c_q[2])
    _loop(8, H + NK, mid)
    _wait(c_inv + c_k[1])

    def inv_s(m):
        zs = []
        for p in range(2):
            rhs = jnp.concatenate([jnp.concatenate([zbuf[t, :, 2 * m + p, c].reshape(N1, 128) for c in range(2)], axis=0)
                                   for t in range(5)], axis=1).astype(bf16)
            zs.append(jnp.dot(gibuf[2 * m + p], rhs, preferred_element_type=f32))
        for t in range(4):
            ln = slice(t * 128, (t + 1) * 128)
            re = [z[:N1, ln] for z in zs]
            im = [jnp.where(lane0, z[:N1, 512:], z[N1:, ln]) if t == 0 else z[N1:, ln] for z in zs]
            lhs = jnp.concatenate([jnp.concatenate(re, axis=0), jnp.concatenate(im, axis=0)], axis=1)
            lbuf[t] = lhs.astype(bf16)

    def inv(m, nxt):
        if nxt:
            wait_if(m == 4, c_v[0])
            wait_if(m == 10, c_v[1])
        ab = []
        for t in range(4):
            v = jnp.dot(lbuf[t], fdibuf[t], preferred_element_type=f32)
            ab.append((v[:, :128], v[:, 128:]))
        if nxt:
            for c in range(3):
                q = 3 * m + c
                relayout((H + NK) // 2 + 1 + q // 2, q % 2,
                         [ab[c][i % 2][8 * (i // 2):8 * (i // 2) + 8] for i in range(32)])
            inv_s(m + 1)
        (p_, q_), (a1, b1), (a2, b2), (a3, b3) = ab
        u0, u2, u4, u6 = p_ + a2, p_ - a2, q_ + b2, q_ - b2
        u1, u3, d, e = a1 + a3, b1 + b3, (a1 - a3) * rt, (b1 - b3) * rt
        u5, u7 = e + d, e - d
        ys = (u0 + u1, u4 + u5, u2 + u3, u6 + u7, u0 - u1, u4 - u5, u2 - u3, u6 - u7)
        for a in range(8):
            y = pltpu.bitcast(ys[a].astype(bf16).astype(f32), u32)
            bxbuf[m, :, a * 128:(a + 1) * 128] = (y[:N1] >> 16) | y[N1:]

    inv_s(0)
    _loop(0, N2 // 2 - 1, lambda m: inv(m, True))
    inv(N2 // 2 - 1, False)
    relayout(3 * NPAIR - 1, 1)
    outu = out_hbm.bitcast(u32)

    c_x = start(x_hbm.at[pl.ds(X1, NSEG - X1)], xbuf.at[pl.ds(X1, NSEG - X1)], 8)
    c_out = [start(bxbuf.at[m], outu.at[:, m, pl.ds(DM, DM)], 0) for m in range(N2 // 2)]
    _wait(c_o)

    hbuf[0:M, :] = membuf[...].astype(f32)
    row = lax.broadcasted_iota(jnp.int32, (L, 128), 0)
    col = lax.broadcasted_iota(jnp.int32, (L, 128), 1)
    mask = (col < L) & ((row < M) | (row >= col))
    scale = DH ** -0.5
    fill = jnp.where(col < L, -1e9 / scale, -jnp.inf)

    def ycopy(s):
        return pltpu.make_async_copy(ybuf.at[s], out_hbm.at[s, :, pl.ds(0, DM)], sems.at[1])

    def step(i, j):
        s, per = i * US + j, NSEG // 2 // US
        hbuf[M:L, :] = xbuf[s].astype(f32)
        st = {}
        acc = [None] * (DM // 128)

        def proj(h):
            hv = hbuf[...]
            if h < NK:
                k = jnp.dot(hv[:L - NP], getw(NPAIR + h // 2, h % 2), preferred_element_type=f32)
                k = jnp.concatenate([k, qkbuf[NPAIR + h // 2, h % 2, i // per, i % per, j * NP:(j + 1) * NP, :]], axis=0)
            else:
                k = jnp.dot(hv, getw(NPAIR + h // 2, h % 2), preferred_element_type=f32)
            q = jnp.dot(hv[:L - NP], getw(h // 2, h % 2), preferred_element_type=f32)
            q = jnp.concatenate([q, qkbuf[h // 2, h % 2, i // per, i % per, j * NP:(j + 1) * NP, :]], axis=0)
            v = jnp.dot(hv, getw(2 * NPAIR + h // 2, h % 2), preferred_element_type=f32)
            zpad = jnp.zeros((128 - L, DH), f32)
            st[h] = (q, jnp.concatenate([k, zpad], axis=0).astype(bf16),
                     jnp.concatenate([v, zpad], axis=0).astype(bf16))

        def qk(h):
            q, kp, vp = st[h]
            st[h] = (lax.dot_general(q, kp, (((1,), (1,)), ((), ())), preferred_element_type=f32), vp)

        def soft(h):
            sc, vp = st[h]
            sc = jnp.where(mask, sc, fill)
            e = jnp.exp2((sc - jnp.max(sc, axis=1, keepdims=True)) * (scale * math.log2(math.e)))
            l = jnp.sum(e, axis=1, keepdims=True)
            r = pl.reciprocal(l, approx=True)
            st[h] = (e, r * (2.0 - l * r), vp)

        def pv(h):
            e, r, vp = st.pop(h)
            obuf[:, h * DH:(h + 1) * DH] = jnp.dot(e, vp, preferred_element_type=f32) * r

        def out(h0, h1, n):
            w = pltpu.bitcast(wobuf[n, h0 * DH // 2:h1 * DH // 2, :], bf16)
            y = jnp.dot(obuf[:, h0 * DH:h1 * DH], w, preferred_element_type=f32)
            acc[n] = y if h0 == 0 else acc[n] + y
            if h1 == H:
                hbuf[0:M, n * 128:(n + 1) * 128] = acc[n][0:M].astype(bf16).astype(f32)
                ybuf[s, :, n * 128:(n + 1) * 128] = acc[n][M:L].astype(bf16)

        fns = dict(proj=proj, qk=qk, soft=soft, pv=pv, out=out)
        for name, *a in _schedule():
            fns[name](*a)
        ycopy(s).start()

    def steps(i):
        for j in range(US):
            step(i, j)

    def phase(ph):
        wait_if(ph == 1, [c_x])
        _loop(ph * (X1 // US), (X1 + ph * (NSEG - X1)) // US, steps)

    _loop(0, 2, phase)
    _wait(c_out)
    _loop(0, NSEG, lambda s: ycopy(s).wait())


@jax.jit
def pallas_concat_heads__memory_aug_recurrent_mem_tr__spectral_gfnet__prompt_kernel(
        A_x, A_mem0, A_Wq, A_Wk, A_Wv, A_Wo, A_seg_len, B_x, B_w_r, B_w_i):
    del A_seg_len
    fd, fdi, g, gi = _consts()
    rw = lambda w: w.reshape(DM // 16, 16, H, DH)
    hbm = pl.BlockSpec(memory_space=pltpu.HBM)
    vm = pltpu.VMEM
    args = (A_x.reshape(NSEG, SEG, DM), A_mem0.reshape(M, DM), rw(A_Wq), rw(A_Wk), rw(A_Wv),
            A_Wo.reshape(H * DH, DM), B_x.reshape(N1, N2, DM), B_w_r.T, B_w_i.T, fd, fdi, g, gi)
    out = pl.pallas_call(
        _kernel,
        out_shape=jax.ShapeDtypeStruct((N1, N2, 2 * DM), bf16),
        in_specs=[hbm] * 13,
        out_specs=hbm,
        scratch_shapes=[
            vm((NSEG, SEG, DM), bf16), vm((M, DM), bf16),
            vm((3 * NPAIR, DM // 16, 16, DH), u32), vm((DM // 128, H * DH // 2, 128), u32),
            vm((L, DM), f32), vm((L, H * DH), f32), vm((NSEG, SEG, DM), bf16),
            vm((N2 // 2, N1, DM), u32), vm((2, S // 128, DM // 4, 128), u32), vm((2, 1, S), bf16), vm((5, 8, N2, 8, 128), u32),
            vm((4, 256, 256), bf16), vm((4, 256, 256), bf16), vm((N2, 128, 128), bf16), vm((N2, 128, 128), bf16),
            vm((5, 8, N2, 2, 8, 128), f32), vm((2, 128, 640), bf16), vm((4, 128, 256), bf16), vm((NSEG, NP, DM), bf16), vm((2, NSEG * NP // 2, DM), f32), vm(((H + NK) // 2, 2, 2, NSEG // 2 // US, US * NP, DH), f32),
            pltpu.SemaphoreType.DMA((16,))],
        compiler_params=pltpu.CompilerParams(vmem_limit_bytes=110 * 1024 * 1024),
    )(*[pltpu.with_memory_space_constraint(jnp.asarray(t), pltpu.HBM) for t in args])
    return out.reshape(1, S, 2 * DM)
```

```python
import functools
import math
import numpy as np
import jax
import jax.numpy as jnp
from jax import lax
from jax.experimental import pallas as pl
from jax.experimental.pallas import tpu as pltpu

S, DM, H, DH, M, SEG = 2048, 1024, 32, 128, 8, 32
L = M + SEG
NSEG = S // SEG
N1, N2 = 64, 32
NPAIR = H // 2
NP, NK = 8, 20
PSTEP = 64
PACE, DIST = 32, 4
US, X1 = 4, 4
f32, bf16, u32 = jnp.float32, jnp.bfloat16, jnp.uint32


def _schedule():
    ev = []
    for h in range(H):
        ev.append(("proj", h))
        g, r = h // 4 - 1, h % 4
        if g >= 0:
            if r == 0:
                ev += [("qk", 4 * g + i) for i in range(4)]
            elif r == 3:
                ev += [("pv", 4 * g + i) for i in range(4)]
            else:
                ev += [("soft", 4 * g + 2 * r - 2), ("soft", 4 * g + 2 * r - 1)]
    o = lambda h0, h1, ns: [("out", h0, h1, n) for n in ns]
    ev += o(0, 8, (0, 1)) + [("qk", h) for h in range(28, 32)] + o(0, 8, (2, 3))
    for i in range(4):
        ev += [("soft", 28 + i)] + o(0, 8, (4 + i,))
    ev += o(8, 16, range(4)) + [("pv", h) for h in range(28, 32)] + o(8, 16, range(4, 8)) + o(16, 32, range(8))
    return ev


_CLS = ((0, 4), (1, 7), (2, 6), (3, 5))
_BETA = {0: 1, 4: -1, 1: -1j, 7: 1j, 2: -1j, 6: 1j, 3: 1j, 5: -1j}


def _consts():
    b = np.arange(128)[:, None]
    fd = np.zeros((4, 256, 256))
    fdi = np.zeros((4, 256, 256))
    for t, cls in enumerate(_CLS):
        k = np.concatenate([c + 8 * np.arange(64) for c in cls])[None, :]
        beta = np.concatenate([np.full(64, _BETA[c], np.complex128) for c in cls])[None, :]
        e = np.exp(-2j * np.pi * ((b * k) % DM) / DM)
        m = np.concatenate([e, beta * e], axis=0)
        re, im = m.real.copy(), m.imag.copy()
        wt = np.full((256,), 2.0)
        if t == 0:
            im[:, 0] = np.tile(np.cos(np.pi * b[:, 0]), 2)
            wt[0] = wt[128] = 1.0
        fd[t] = np.concatenate([re, im], axis=1)
        fdi[t] = fd[t].T * wt[:, None] / (S * DM)
    n2 = np.arange(N2)[:, None, None]
    k1 = np.arange(N1)[None, :, None]
    n1 = np.arange(N1)[None, None, :]
    a = 2 * np.pi * ((k1 * (N2 * n1 + n2)) % S) / S
    c, s = np.cos(a), -np.sin(a)
    g = np.concatenate([np.concatenate([c, -s], axis=2), np.concatenate([s, c], axis=2)], axis=1)
    gi = np.transpose(g, (0, 2, 1))
    cast = lambda t: np.ascontiguousarray(t).astype(np.float32).astype(jnp.bfloat16)
    return cast(fd), cast(fdi), cast(g), cast(gi)


def _tw(z, k, n):
    k %= n
    zr, zi = z
    if k == 0:
        return z
    if 4 * k == n:
        return (zi, -zr)
    if 2 * k == n:
        return (-zr, -zi)
    if 4 * k == 3 * n:
        return (-zi, zr)
    c, s = math.cos(2 * math.pi * k / n), -math.sin(2 * math.pi * k / n)
    if (8 * k) % n == 0:
        r = math.sqrt(0.5)
        if 8 * k == n:
            return ((zr + zi) * r, (zi - zr) * r)
        if 8 * k == 3 * n:
            return ((zi - zr) * r, (zr + zi) * (-r))
    return (zr * c - zi * s, zr * s + zi * c)


def _fft(x):
    n = len(x)
    if n == 1:
        return x
    if n == 2:
        (ar, ai), (br, bi) = x
        return [(ar + br, ai + bi), (ar - br, ai - bi)]
    e, o1, o3 = _fft(x[0::2]), _fft(x[1::4]), _fft(x[3::4])
    out = [None] * n
    q = n // 4
    for k in range(q):
        t1, t3 = _tw(o1[k], k, n), _tw(o3[k], 3 * k, n)
        sr, si = t1[0] + t3[0], t1[1] + t3[1]
        dr, di = t1[0] - t3[0], t1[1] - t3[1]
        out[k] = (e[k][0] + sr, e[k][1] + si)
        out[k + 2 * q] = (e[k][0] - sr, e[k][1] - si)
        out[k + q] = (e[k + q][0] + di, e[k + q][1] - dr)
        out[k + 3 * q] = (e[k + q][0] - di, e[k + q][1] + dr)
    return out


def _ifft(x):
    return [(b, a) for a, b in _fft([(b, a) for a, b in x])]


def _loop(lo, hi, fn):
    def body(i, c):
        fn(i)
        return c
    lax.fori_loop(lo, hi, body, 0)


def _wait(cs):
    for c in cs:
        c.wait()


def _lo(w):
    return pltpu.bitcast(w << 16, f32)


def _hi(w):
    return pltpu.bitcast(w & jnp.uint32(0xFFFF0000), f32)


def _kernel(x_hbm, mem_hbm, wq_hbm, wk_hbm, wv_hbm, wo_hbm, bx_hbm, wr_hbm, wi_hbm,
            fd_hbm, fdi_hbm, g_hbm, gi_hbm, out_hbm,
            xbuf, membuf, wbuf0, wbuf1, wobuf, hbuf, obuf, ybuf,
            bxbuf, wtbuf, wnbuf, wpbuf, fdbuf, fdibuf, gbuf, gibuf, zbuf, rbuf, lbuf, xqbuf, xfbuf, qkbuf, sems):
    def start(src, dst, i):
        c = pltpu.make_async_copy(src, dst, sems.at[i])
        c.start()
        return c

    bxu = bx_hbm.bitcast(u32)

    def load_f(m0, m1, sem):
        gs = pl.ds(2 * m0, 2 * (m1 - m0))
        return ([start(g_hbm.at[gs], gbuf.at[gs], sem)]
                + [start(bxu.at[:, m, :], bxbuf.at[m], sem) for m in range(m0, m1)])

    c_f = [start(fd_hbm, fdbuf, 0)] + load_f(0, 2, 0)
    c_f2 = [load_f(2, 4, 1), load_f(4, 8, 13), load_f(8, 16, 14)]

    wbufs = (wbuf0, wbuf1)

    def load_w(t, j0, j1, sem):
        wu = (wq_hbm, wk_hbm, wv_hbm)[t].bitcast(u32)
        return [start(wu.at[:, :, j, :], wbufs[j % 2].at[(t * NPAIR + j) // 2], sem) for j in range(j0, j1)]

    def getw(par, e, p):
        w = wbufs[par][e, :, pl.ds(p * 8, 8), :]
        return pltpu.bitcast(w.reshape(DM // 2, DH), bf16)

    def relayout(par, e, half, pace=None):
        wbuf = wbufs[par]
        for i in range(32):
            g = 32 * half + i
            a = wbuf[e, g, pl.ds(0, 8, stride=2), :]
            b = wbuf[e, g, pl.ds(1, 8, stride=2), :]
            if pace is not None:
                a = jnp.where(pace[0] < 0, pltpu.bitcast(pace[1][i], u32), a)
            wbuf[e, g, 0:8, :] = (a & jnp.uint32(0xFFFF)) | (b << 16)
            wbuf[e, g, 8:16, :] = (a >> 16) | (b & jnp.uint32(0xFFFF0000))

    def wait_if(cond, cs):
        @pl.when(cond)
        def _():
            for c in cs:
                c.wait()

    lane0 = lax.broadcasted_iota(jnp.int32, (N1, 128), 1) == 0
    rt = math.sqrt(0.5)

    def fwd_d(m):
        w = bxbuf[m]
        xs = [jnp.concatenate([_lo(w[:, a * 128:(a + 1) * 128]), _hi(w[:, a * 128:(a + 1) * 128])], axis=0)
              for a in range(8)]
        u0, u1, u2, u3 = xs[0] + xs[4], xs[0] - xs[4], xs[2] + xs[6], xs[2] - xs[6]
        u4, u5, u6, u7 = xs[1] + xs[5], xs[1] - xs[5], xs[3] + xs[7], xs[3] - xs[7]
        d, e = (u5 - u7) * rt, (u5 + u7) * rt
        ab = ((u0 + u2, u4 + u6), (u1 + d, u3 + e), (u0 - u2, u4 - u6), (u1 - d, u3 - e))
        z = [jnp.dot(jnp.concatenate(ab[t], axis=1).astype(bf16), fdbuf[t], preferred_element_type=f32)
             for t in range(4)]
        for p in range(2):
            rows = slice(p * N1, (p + 1) * N1)
            zi0 = z[0][rows, 128:]
            top = [z[t][rows, :128] for t in range(4)] + [jnp.where(lane0, zi0, 0.0)]
            bot = [jnp.where(lane0, 0.0, zi0)] + [z[t][rows, 128:] for t in range(1, 4)] + [jnp.zeros((N1, 128), f32)]
            rhs = jnp.concatenate([jnp.concatenate(top, axis=1), jnp.concatenate(bot, axis=1)], axis=0)
            rbuf[p] = rhs.astype(bf16)

    def fwd_s(m):
        for p in range(2):
            y = jnp.dot(gbuf[2 * m + p], rbuf[p], preferred_element_type=f32)
            for t in range(5):
                for c in range(2):
                    zbuf[t, :, 2 * m + p, c] = y[c * N1:(c + 1) * N1, t * 128:(t + 1) * 128].reshape(8, 8, 128)

    def fwd(m):
        for c, m0 in zip(c_f2, (2, 4, 8)):
            wait_if(m == m0, c)
        fwd_s(m - 1)
        fwd_d(m)

    def permute_w(jt):
        def put(i, v):
            v = v.T
            for c in range(2):
                wpbuf[i, :, 2 * jt + c] = v[c * N1:(c + 1) * N1].reshape(8, 8, 128)
        ln = pl.ds(jt * 128, 128)
        for i in range(2):
            p = [wtbuf[i, jt, pl.ds(c, 64, stride=4), :] for c in range(4)]
            lo, hi = jnp.uint32(0xFFFF), jnp.uint32(0xFFFF0000)
            put(2 * i, jnp.concatenate([p[0], (p[2] & lo) | (p[3] & hi)], axis=0))
            put(2 * i + 1, jnp.concatenate([p[1], (p[3] & lo) | (p[2] & hi)], axis=0))
        nr = pltpu.bitcast(wnbuf[0, :, ln].astype(f32), u32)
        ni = pltpu.bitcast(wnbuf[1, :, ln].astype(f32), u32)
        put(4, jnp.broadcast_to((nr >> 16) | ni, (128, 128)))

    c_q = [[start(x_hbm.at[:, pl.ds(SEG - NP, NP), :], xqbuf, 4)] + load_w(0, 0, 5, 4)]
    c_w = []
    for i, w in enumerate((wr_hbm, wi_hbm)):
        wu = w.at[pl.ds(0, DM // 2), :].bitcast(u32)
        c_w += [start(wu.at[:, pl.ds(j * 128, 128)], wtbuf.at[i, j], 2) for j in range(S // 128)]
        c_w.append(start(w.at[pl.ds(DM // 2, 1), :], wnbuf.at[i], 2))

    _wait(c_f)
    fwd_d(0)
    _loop(1, N2 // 2, fwd)
    fwd_s(N2 // 2 - 1)
    c_q += [load_w(0, 5, 7, 5)]

    def mid_pieces(g, t, res):
        gate = [len(res) - DIST - 1]

        def lds(ns):
            z = [(zbuf[t, g, n, 0], zbuf[t, g, n, 1]) for n in ns]
            gate.append(max(gate[-1] + 1, len(res) - DIST))
            if 0 <= gate[-1] < len(res):
                z[0] = (jnp.where(t < 0, res[gate[-1]], z[0][0]), z[0][1])
                z[1] = (z[1][0], jnp.where(t < 0, res[gate[-1]], z[1][1]))
            return z
        nyq = t // 4
        ir, ii = t // 2 + 2 * nyq, t // 2 + 2
        sr = (16 * (1 - t % 2)).astype(u32)
        si = (16 * (1 - t % 2 - nyq)).astype(u32)
        half = lambda w, sh: pltpu.bitcast((w << sh) & jnp.uint32(0xFFFF0000), f32)

        def st(n, z):
            zbuf[t, g, n, 0] = z[0]
            zbuf[t, g, n, 1] = z[1]

        def p1(b):
            y = _fft(lds([4 * a + b for a in range(8)]))
            for ka in range(8):
                st(4 * ka + b, _tw(y[ka], b * ka, N2))

        def p2(ka):
            y = _fft(lds([4 * ka + b for b in range(4)]))
            for kb in range(4):
                wr, wi = half(wpbuf[ir, g, ka + 8 * kb], sr), half(wpbuf[ii, g, ka + 8 * kb], si)
                yr, yi = y[kb]
                y[kb] = (yr * wr - yi * wi, yr * wi + yi * wr)
            y = _ifft(y)
            for b in range(4):
                st(4 * ka + b, _tw(y[b], -b * ka, N2))

        def p3(b):
            y = _ifft(lds([4 * ka + b for ka in range(8)]))
            for a in range(8):
                st(4 * a + b, y[a])

        P = functools.partial
        return [P(p1, b) for b in range(4)] + [P(p2, k) for k in range(8)] + [P(p3, b) for b in range(4)]

    def pre_pieces(par, e, half, step, res):
        def piece(p, r):
            y = jnp.dot(xfbuf[half, r:r + step, :], getw(par, e, p), preferred_element_type=f32)
            res.extend(y[c:c + 8] for c in range(0, step, PACE))
            n = US * NP
            qkbuf[par, e, p, half, r // n:(r + step) // n] = y.reshape(step // n, n, DH)
        return [functools.partial(piece, p, r) for p in range(2) for r in range(0, NSEG * NP // 2, step)]

    def pre(e, side, step):
        res = []
        for j in range(4):
            par, half = j // 2, j % 2
            pp, sp = pre_pieces(par, e, half, step, res), side(j, res)
            k = len(sp) // len(pp)
            for c, p in enumerate(pp):
                p()
                for f in sp[c * k:(c + 1) * k]:
                    f()
            relayout(1 - par, e + par, half)

    def mid(i):
        wait_if(i == 2, c_q[3])
        wait_if(i == 4, c_k[0])
        wait_if(i == 7, c_k[1])
        pre(3 + i, lambda j, res: mid_pieces((4 * i + j) // 5, (4 * i + j) % 5, res), PSTEP)

    _wait(c_q[0])
    xfbuf[...] = xqbuf[...].astype(f32).reshape(2, NSEG * NP // 2, DM)
    relayout(0, 0, 0)
    relayout(0, 0, 1)
    _loop(0, 2, lambda e: pre(e, lambda j, res: [], 256))
    c_q += [load_w(0, 7, 11, 6), load_w(0, 11, 16, 15)]
    c_k = [load_w(1, 0, 5, 9), load_w(1, 5, 16, 10)]
    c_inv = [start(fdi_hbm, fdibuf, 3), start(gi_hbm, gibuf, 3)]
    c_v = [load_w(2, 0, 8, 11), load_w(2, 8, 16, 12)]
    wou = wo_hbm.bitcast(u32)
    c_o = [start(wou.at[:, pl.ds(n * 128, 128)], wobuf.at[n], 7) for n in range(DM // 128)]
    c_o.append(start(mem_hbm, membuf, 7))
    c_o.append(start(x_hbm.at[pl.ds(0, X1)], xbuf.at[pl.ds(0, X1)], 7))

    _wait(c_w + c_q[1])
    pre(2, lambda j, res: [functools.partial(permute_w, 4 * j + c) for c in range(4)], 256)

    _wait(c_q[2])
    _loop(0, 10, mid)
    _wait(c_inv)

    def inv_s(m):
        zs = []
        for p in range(2):
            rhs = jnp.concatenate([jnp.concatenate([zbuf[t, :, 2 * m + p, c].reshape(N1, 128) for c in range(2)], axis=0)
                                   for t in range(5)], axis=1).astype(bf16)
            zs.append(jnp.dot(gibuf[2 * m + p], rhs, preferred_element_type=f32))
        for t in range(4):
            ln = slice(t * 128, (t + 1) * 128)
            re = [z[:N1, ln] for z in zs]
            im = [jnp.where(lane0, z[:N1, 512:], z[N1:, ln]) if t == 0 else z[N1:, ln] for z in zs]
            lhs = jnp.concatenate([jnp.concatenate(re, axis=0), jnp.concatenate(im, axis=0)], axis=1)
            lbuf[t] = lhs.astype(bf16)

    def inv(m, nxt, chunks):
        ab = []
        for t in range(4):
            v = jnp.dot(lbuf[t], fdibuf[t], preferred_element_type=f32)
            ab.append((v[:, :128], v[:, 128:]))
        for c, (par, e, half) in enumerate(chunks):
            relayout(par, e, half, (m, [ab[c % 4][i % 2][8 * (i // 2):8 * (i // 2) + 8] for i in range(32)]))
        if nxt:
            inv_s(m + 1)
        (p_, q_), (a1, b1), (a2, b2), (a3, b3) = ab
        u0, u2, u4, u6 = p_ + a2, p_ - a2, q_ + b2, q_ - b2
        u1, u3, d, e = a1 + a3, b1 + b3, (a1 - a3) * rt, (b1 - b3) * rt
        u5, u7 = e + d, e - d
        ys = (u0 + u1, u4 + u5, u2 + u3, u6 + u7, u0 - u1, u4 - u5, u2 - u3, u6 - u7)
        for a in range(8):
            y = pltpu.bitcast(ys[a].astype(bf16).astype(f32), u32)
            bxbuf[m, :, a * 128:(a + 1) * 128] = (y[:N1] >> 16) | y[N1:]

    inv_s(0)

    def invs(i):
        wait_if(i == 1, c_v[0])
        wait_if(i == 3, c_v[1])
        ch = [(1 - v % 2, 13 + 2 * i + (v + 1) // 2, half) for v in range(4) for half in range(2)]
        for j in range(3):
            inv(3 * i + j, True, ch[3 * j:3 * j + 3])
    _loop(0, 5, invs)
    _loop(N2 // 2 - 1, N2 // 2, lambda m: inv(m, False, [(u % 2, u // 2, half) for u in (47,) for half in range(2)]))
    outu = out_hbm.bitcast(u32)

    c_x = start(x_hbm.at[pl.ds(X1, NSEG - X1)], xbuf.at[pl.ds(X1, NSEG - X1)], 8)
    c_out = [start(bxbuf.at[m], outu.at[:, m, pl.ds(DM, DM)], 0) for m in range(N2 // 2)]
    _wait(c_o)

    hbuf[0:M, :] = membuf[...].astype(f32)
    row = lax.broadcasted_iota(jnp.int32, (L, 128), 0)
    col = lax.broadcasted_iota(jnp.int32, (L, 128), 1)
    mask = (col < L) & ((row < M) | (row >= col))
    scale = DH ** -0.5
    fill = jnp.where(col < L, -1e9 / scale, -jnp.inf)

    def ycopy(s):
        return pltpu.make_async_copy(ybuf.at[s], out_hbm.at[s, :, pl.ds(0, DM)], sems.at[1])

    def step(i, j):
        s, per = i * US + j, NSEG // 2 // US
        hbuf[M:L, :] = xbuf[s].astype(f32)
        st = {}
        acc = [None] * (DM // 128)

        def proj(h):
            hv = hbuf[...]
            if h < NK:
                k = jnp.dot(hv[:L - NP], getw(h // 2 % 2, (NPAIR + h // 2) // 2, h % 2), preferred_element_type=f32)
                k = jnp.concatenate([k, qkbuf[h // 2 % 2, (NPAIR + h // 2) // 2, h % 2, i // per, i % per, j * NP:(j + 1) * NP, :]], axis=0)
            else:
                k = jnp.dot(hv, getw(h // 2 % 2, (NPAIR + h // 2) // 2, h % 2), preferred_element_type=f32)
            q = jnp.dot(hv[:L - NP], getw(h // 2 % 2, h // 4, h % 2), preferred_element_type=f32)
            q = jnp.concatenate([q, qkbuf[h // 2 % 2, h // 4, h % 2, i // per, i % per, j * NP:(j + 1) * NP, :]], axis=0)
            v = jnp.dot(hv, getw(h // 2 % 2, (2 * NPAIR + h // 2) // 2, h % 2), preferred_element_type=f32)
            zpad = jnp.zeros((128 - L, DH), f32)
            st[h] = (q, jnp.concatenate([k, zpad], axis=0).astype(bf16),
                     jnp.concatenate([v, zpad], axis=0).astype(bf16))

        def qk(h):
            q, kp, vp = st[h]
            st[h] = (lax.dot_general(q, kp, (((1,), (1,)), ((), ())), preferred_element_type=f32), vp)

        def soft(h):
            sc, vp = st[h]
            sc = jnp.where(mask, sc, fill)
            e = jnp.exp2((sc - jnp.max(sc, axis=1, keepdims=True)) * (scale * math.log2(math.e)))
            l = jnp.sum(e, axis=1, keepdims=True)
            r = pl.reciprocal(l, approx=True)
            st[h] = (e, r * (2.0 - l * r), vp)

        def pv(h):
            e, r, vp = st.pop(h)
            obuf[:, h * DH:(h + 1) * DH] = jnp.dot(e, vp, preferred_element_type=f32) * r

        def out(h0, h1, n):
            w = pltpu.bitcast(wobuf[n, h0 * DH // 2:h1 * DH // 2, :], bf16)
            y = jnp.dot(obuf[:, h0 * DH:h1 * DH], w, preferred_element_type=f32)
            acc[n] = y if h0 == 0 else acc[n] + y
            if h1 == H:
                hbuf[0:M, n * 128:(n + 1) * 128] = acc[n][0:M].astype(bf16).astype(f32)
                ybuf[s, :, n * 128:(n + 1) * 128] = acc[n][M:L].astype(bf16)

        fns = dict(proj=proj, qk=qk, soft=soft, pv=pv, out=out)
        for name, *a in _schedule():
            fns[name](*a)
        ycopy(s).start()

    def steps(i):
        for j in range(US):
            step(i, j)

    def phase(ph):
        wait_if(ph == 1, [c_x])
        _loop(ph * (X1 // US), (X1 + ph * (NSEG - X1)) // US, steps)

    _loop(0, 2, phase)
    _wait(c_out)
    _loop(0, NSEG, lambda s: ycopy(s).wait())


@jax.jit
def pallas_concat_heads__memory_aug_recurrent_mem_tr__spectral_gfnet__prompt_kernel(
        A_x, A_mem0, A_Wq, A_Wk, A_Wv, A_Wo, A_seg_len, B_x, B_w_r, B_w_i):
    del A_seg_len
    fd, fdi, g, gi = _consts()
    rw = lambda w: w.reshape(DM // 16, 16, H, DH)
    hbm = pl.BlockSpec(memory_space=pltpu.HBM)
    vm = pltpu.VMEM
    args = (A_x.reshape(NSEG, SEG, DM), A_mem0.reshape(M, DM), rw(A_Wq), rw(A_Wk), rw(A_Wv),
            A_Wo.reshape(H * DH, DM), B_x.reshape(N1, N2, DM), B_w_r.T, B_w_i.T, fd, fdi, g, gi)
    out = pl.pallas_call(
        _kernel,
        out_shape=jax.ShapeDtypeStruct((N1, N2, 2 * DM), bf16),
        in_specs=[hbm] * 13,
        out_specs=hbm,
        scratch_shapes=[
            vm((NSEG, SEG, DM), bf16), vm((M, DM), bf16),
            vm((3 * NPAIR // 2, DM // 16, 16, DH), u32), vm((3 * NPAIR // 2, DM // 16, 16, DH), u32), vm((DM // 128, H * DH // 2, 128), u32),
            vm((L, DM), f32), vm((L, H * DH), f32), vm((NSEG, SEG, DM), bf16),
            vm((N2 // 2, N1, DM), u32), vm((2, S // 128, DM // 4, 128), u32), vm((2, 1, S), bf16), vm((5, 8, N2, 8, 128), u32),
            vm((4, 256, 256), bf16), vm((4, 256, 256), bf16), vm((N2, 128, 128), bf16), vm((N2, 128, 128), bf16),
            vm((5, 8, N2, 2, 8, 128), f32), vm((2, 128, 640), bf16), vm((4, 128, 256), bf16), vm((NSEG, NP, DM), bf16), vm((2, NSEG * NP // 2, DM), f32), vm((2, (H + NK) // 4, 2, 2, NSEG // 2 // US, US * NP, DH), f32),
            pltpu.SemaphoreType.DMA((16,))],
        compiler_params=pltpu.CompilerParams(vmem_limit_bytes=110 * 1024 * 1024),
    )(*[pltpu.with_memory_space_constraint(jnp.asarray(t), pltpu.HBM) for t in args])
    return out.reshape(1, S, 2 * DM)
```
